```python
import jax
import jax.numpy as jnp

def _softmax(x, axis=-1):
    return jax.nn.softmax(x, axis=axis)
def _gelu(x):
    return jax.nn.gelu(x, approximate=True)
def _silu(x):
    return jax.nn.silu(x)
def _sigmoid(x):
    return jax.nn.sigmoid(x)
def _layernorm(x, axis=-1, eps=1e-5):
    m = jnp.mean(x, axis=axis, keepdims=True)
    v = jnp.var(x, axis=axis, keepdims=True)
    return (x - m) / jnp.sqrt(v + eps)
def _scatter_add(tgt, idx, src, axis=0):
    return tgt.at[idx].add(src)
def _segment_sum(src, seg, n):
    return jax.ops.segment_sum(src, seg, n)
class _Rng:
    def __init__(self, key):
        self._k = key
    def _next(self):
        self._k, sub = jax.random.split(self._k)
        return sub
    def normal(self, shape):
        return jax.random.normal(self._next(), shape, dtype=jnp.bfloat16)
    def randint(self, lo, hi, shape):
        return jax.random.randint(self._next(), shape, lo, hi, dtype=jnp.int32)
    def uniform(self, shape, lo=0.0, hi=1.0):
        return jax.random.uniform(self._next(), shape, jnp.bfloat16, lo, hi)
    def permutation(self, n):
        return jax.random.permutation(self._next(), n)


kernel_name = 'parallel_sum__ssm_conv_h3__dense_activation_gelu__prompt'

def setup_inputs():
    _rng = _Rng(jax.random.key(int.from_bytes(__import__("os").urandom(4), "little")))
    _w = (lambda a: (lambda t: t.astype(jnp.bfloat16) if jnp.issubdtype(t.dtype, jnp.floating) else t)(jnp.asarray(a)))
    def _A_setup():
        B, S, D = 1, 2048, 640
        ks = 4
        return {
            "q": _w((lambda *s: _rng.normal(s) * 0.05)(B, S, D)),
            "k": _w((lambda *s: _rng.normal(s) * 0.05)(B, S, D)),
            "v": _w((lambda *s: _rng.normal(s) * 0.05)(B, S, D)),
            "shift_k": _w((lambda *s: _rng.normal(s) * 0.05)(D, ks) * 0.5),
            "ssm_k": _w((lambda *s: _rng.normal(s) * 0.05)(D, S) * (1.0 / S ** 0.5)),
            "ssm_D": _w((lambda *s: _rng.normal(s) * 0.05)(D)),
        }
    _A_in = _A_setup()

    def _B_setup():
        B, S, D, F = 1, 2048, 640, 1728
        return {
            "x": _w((lambda *s: _rng.normal(s) * 0.05)(B, S, D)),
            "w1": _w((lambda *s: _rng.normal(s) * 0.05)(D, F) * (D ** -0.5)),
            "b1": _w((lambda *s: _rng.normal(s) * 0.05)(F) * 0.01),
            "w2": _w((lambda *s: _rng.normal(s) * 0.05)(F, D) * (F ** -0.5)),
            "b2": _w((lambda *s: _rng.normal(s) * 0.05)(D) * 0.01),
        }
    _B_in = _B_setup()

    return {
        "A_q": _A_in["q"],
        "A_k": _A_in["k"],
        "A_v": _A_in["v"],
        "A_shift_k": _A_in["shift_k"],
        "A_ssm_k": _A_in["ssm_k"],
        "A_ssm_D": _A_in["ssm_D"],
        "B_x": _B_in["x"],
        "B_w1": _B_in["w1"],
        "B_b1": _B_in["b1"],
        "B_w2": _B_in["w2"],
        "B_b2": _B_in["b2"],
    }

def reference(A_q, A_k, A_v, A_shift_k, A_ssm_k, A_ssm_D, B_x, B_w1, B_b1, B_w2, B_b2):
    def _A_ref(q, k, v, shift_k, ssm_k, ssm_D):
        B, S, D = q.shape
        ks = shift_k.shape[-1]
        k_pad = jnp.pad(k, ((0, 0), (ks - 1, 0), (0, 0)))
        k_shift = jnp.zeros_like(k)
        for t in range(ks):
            k_shift = k_shift + k_pad[:, t:t + S, :] * shift_k[:, ks - 1 - t][None, None, :]
        kv = k_shift * v
        L = 2 * S
        kv_pad = jnp.pad(kv, ((0, 0), (0, S), (0, 0)))
        kf_pad = jnp.pad(ssm_k, ((0, 0), (0, S)))
        kv_f = (lambda x, axes=(-2,-1): jnp.fft.rfft2(x.astype(jnp.float32), axes=axes))(kv_pad[:, None, :, :], axes=(1, 2))
        kf_f = (lambda x, axes=(-2,-1): jnp.fft.rfft2(x.astype(jnp.float32), axes=axes))(kf_pad[:, None, :], axes=(1, 2))
        kf_f = (lambda x, *d: x.transpose(*d))(kf_f, 1, 2, 0)
        y_f = kv_f * kf_f[None, :, :, :]
        y = (lambda x, s, axes=(-2,-1): jnp.fft.irfft2(x, s=s, axes=axes).astype(jnp.bfloat16))(y_f, (1, L), axes=(1, 2))[:, 0, :S, :]
        y = y + kv * ssm_D[None, None, :]
        return q * y

    def _B_ref(x, w1, b1, w2, b2):
        h = jnp.einsum("bsd,df->bsf", x, w1) + b1
        h = _gelu(h)
        return jnp.einsum("bsf,fd->bsd", h, w2) + b2

    x = A_q
    xn = _layernorm(x, axis=-1)
    return x + _A_ref(xn, A_k, A_v, A_shift_k, A_ssm_k, A_ssm_D) + _B_ref(xn, B_w1, B_b1, B_w2, B_b2)
```

```python
import functools
import numpy as np
import jax
import jax.numpy as jnp
import jax.experimental.pallas as pl
import jax.experimental.pallas.tpu as pltpu

S, D, F, KS = 2048, 640, 1728, 4
FP = 1792
N1, N2 = 128, 16
CT = 128
NCT = D // CT
MP, MM = 448, 320
ME = MM
FC = 256
MH = max(MP, MM, ME) // 2
NT = FP // CT
B_HID = 0
B_A = NT * MH
B_ROWS = B_A + 2 * N2 * 2 * N1
TS = S // 2
C_K, C_V, C_F, C_BASE = 0, NCT * TS, 2 * NCT * TS, 3 * NCT * TS
C_ROWS = 4 * NCT * TS
assert MP + (NCT - 1) * MM + ME == S


def _dft_consts():
    n1 = np.arange(N1)
    k1 = np.arange(N1)
    g = np.zeros((N2, 2 * N1, N1), np.float64)
    for n2 in range(N2):
        t = N2 * n1 + n2
        ph = np.pi * t[None, :] / (2 * S) - 2 * np.pi * ((t[None, :] * k1[:, None]) % S) / S
        g[n2, :N1] = np.cos(ph)
        g[n2, N1:] = np.sin(ph)
    g = g.reshape(N2, 2, N1 // 8, 8, N1).transpose(0, 2, 1, 3, 4).reshape(N2, 2 * N1, N1)
    h = np.transpose(g, (0, 2, 1)) / S

    def pack(m):
        u = np.ascontiguousarray(m).astype(jnp.bfloat16).view(np.uint16).astype(np.uint32)
        return u[:, 0::2, :] | (u[:, 1::2, :] << 16)

    return pack(g), pack(h)


_G, _H = _dft_consts()


def _cmul_const(re, im, e):
    e = e % 16
    if e == 0:
        return re, im
    c = float(np.cos(2 * np.pi * e / 16))
    s = float(-np.sin(2 * np.pi * e / 16))
    if e % 2 == 0:
        if c * s > 0:
            return (re - im) * c, (re + im) * c
        return (re + im) * c, (im - re) * c
    return re * c - im * s, re * s + im * c


def _r4(x, sign, rot2=False):
    (ar, ai), (br, bi), (cr, ci), (dr, di) = x
    if not rot2:
        t0r, t0i = ar + cr, ai + ci
        t1r, t1i = ar - cr, ai - ci
    elif sign > 0:
        t0r, t0i = ar + ci, ai - cr
        t1r, t1i = ar - ci, ai + cr
    else:
        t0r, t0i = ar - ci, ai + cr
        t1r, t1i = ar + ci, ai - cr
    t2r, t2i = br + dr, bi + di
    t3r, t3i = br - dr, bi - di
    y0 = (t0r + t2r, t0i + t2i)
    y2 = (t0r - t2r, t0i - t2i)
    ym = (t1r + t3i, t1i - t3r)
    yp = (t1r - t3i, t1i + t3r)
    if sign > 0:
        return [y0, ym, y2, yp]
    return [y0, yp, y2, ym]


def _tw(y, b, c, sign):
    return y if b * c == 4 else _cmul_const(*y, sign * b * c)


def _unpack(u):
    lo = pltpu.bitcast(u << 16, jnp.float32)
    hi = pltpu.bitcast(u & jnp.uint32(0xFFFF0000), jnp.float32)
    return lo, hi


def _gelu(h):
    c0 = float(np.sqrt(2 / np.pi))
    c1 = c0 * 0.044715
    u = h * (c0 + c1 * (h * h))
    hh = 0.5 * h
    return hh + hh * jnp.tanh(u)


def _kernel(q_hbm, k_hbm, v_hbm, sk_hbm, f_hbm, d_hbm, w1_hbm, b1_hbm, w2_hbm, b2_hbm, g_hbm, h_hbm,
            o_hbm,
            q_ref, pc_ref, w1_ref, w2_ref, g32, h32, o_ref, xn32, pb32, r32, b_ref, t_ref,
            sk_ref, d_ref, b1_ref, b2_ref, prm_ref, y_ref, sems):
    bf = jnp.bfloat16
    u32 = jnp.uint32
    pc32, o32, w132, w232 = (r.bitcast(u32) for r in (pc_ref, o_ref, w1_ref, w2_ref))
    asf = lambda x: pltpu.bitcast(x, jnp.float32)
    asbf = lambda x: pltpu.bitcast(x, bf)
    as32 = lambda x: pltpu.bitcast(x, u32)

    nsem = [0]

    def copy(src, dst):
        c = pltpu.make_async_copy(src, dst, sems.at[nsem[0]])
        nsem[0] += 1
        return c

    c_q0 = copy(q_hbm.at[0:MP], q_ref.at[0:MP])
    c_small = [copy(sk_hbm, sk_ref), copy(d_hbm, d_ref), copy(b1_hbm, b1_ref), copy(b2_hbm, b2_ref)]
    c_w1 = [[copy(w1_hbm.at[f0:f1, c * CT:(c + 1) * CT], w1_ref.at[c, f0:f1]) for c in range(NCT)]
            for f0, f1 in ((0, FC), (FC, 3 * FC), (3 * FC, F))]
    c_w2 = [copy(w2_hbm.at[:, c * CT:(c + 1) * CT], w2_ref.at[c, 0:F]) for c in range(NCT)]
    c_g = copy(g_hbm, g32)
    c_h = copy(h_hbm, h32)
    kvf_base = nsem[0]

    def kvf_start(j):
        al = (lambda x, n: x) if isinstance(j, int) else pl.multiple_of
        c0 = al(j * CT, CT)
        pltpu.make_async_copy(k_hbm.at[:, pl.ds(c0, CT)], pc_ref.at[pl.ds(al(2 * (C_K + j * TS), S), S)],
                              sems.at[kvf_base + 3 * j]).start()
        pltpu.make_async_copy(v_hbm.at[:, pl.ds(c0, CT)], pc_ref.at[pl.ds(al(2 * (C_V + j * TS), S), S)],
                              sems.at[kvf_base + 3 * j + 1]).start()
        for m in range(S // CT):
            pltpu.make_async_copy(f_hbm.at[pl.ds(c0, CT), m * CT:(m + 1) * CT],
                                  pc_ref.at[pl.ds(al(2 * (C_F + j * TS) + m * CT, CT), CT)],
                                  sems.at[kvf_base + 3 * j + 2]).start()

    def kvf_wait(j):
        for i, c in enumerate((C_K, C_V, C_F)):
            r0 = 2 * (c + j * TS)
            dst = pc_ref.at[pl.ds(r0 if isinstance(j, int) else pl.multiple_of(r0, S), S)]
            pltpu.make_async_copy(dst, dst, sems.at[kvf_base + 3 * j + i]).wait()

    def q_copy(j):
        r0 = MP + j * MM if isinstance(j, int) else pl.multiple_of(MP + j * MM, 16)
        return pltpu.make_async_copy(q_hbm.at[pl.ds(r0, MM)], q_ref.at[pl.ds(r0, MM)], sems.at[kvf_base + 3 * NCT + j])

    nsem[0] += 4 * NCT
    for c in [c_q0] + c_w1[0] + c_small:
        c.start()

    w1_ref[:, F:FP, :] = jnp.zeros((NCT, FP - F, CT), bf)
    w2_ref[:, F:FP, :] = jnp.zeros((NCT, FP - F, CT), bf)
    for c in c_small:
        c.wait()
    b1 = b1_ref[...].astype(jnp.float32).reshape(1, F)
    b1 = jnp.concatenate([b1, jnp.zeros((1, FP - F), jnp.float32)], axis=1)
    b2 = b2_ref[...].astype(jnp.float32).reshape(1, D)
    dd = d_ref[...].astype(jnp.float32).reshape(1, D)
    skt = sk_ref[...].astype(jnp.float32)
    for j in range(NCT):
        prm_ref[j, 0:KS, :] = skt[:, j * CT:(j + 1) * CT]
        prm_ref[j, KS:KS + 1, :] = dd[:, j * CT:(j + 1) * CT]

    def drain(q, n):
        for _ in range(n):
            if q:
                q.pop(0)()

    def share(n, i, parts):
        return (i + 1) * n // parts - i * n // parts

    def mlp_pieces(r0, m, hid32, hid0):
        rows = pl.ds(r0, m)
        h0 = r0 // 2 if isinstance(r0, int) else pl.multiple_of(r0 // 2, 8)
        ng = m // 16

        def ln():
            x = q_ref[rows, :].astype(jnp.float32)
            mu = jnp.mean(x, axis=-1, keepdims=True)
            xc = x - mu
            var = jnp.mean(xc * xc, axis=-1, keepdims=True)
            xn = as32((xc * jax.lax.rsqrt(var + 1e-5)).astype(bf))
            for c in range(NCT):
                xn32[c, pl.ds(h0, m // 2), :] = xn[:, c * CT:(c + 1) * CT]

        def mm1(t, side, n):
            xn = asbf(jnp.concatenate([xn32[c, pl.ds(h0, m // 2), :] for c in range(NCT)], axis=1))
            w = asbf(jnp.concatenate([w132[c, t * CT // 2:(t + 1) * CT // 2, :] for c in range(NCT)], axis=1))
            hh = jax.lax.dot_general(xn, w, (((1,), (1,)), ((), ())),
                                     preferred_element_type=jnp.float32) + b1[:, t * CT:(t + 1) * CT]
            hh = as32(_gelu(hh).astype(bf))
            for g in range(ng):
                hid32[pl.ds(hid0 + t * MH + 8 * g, 8), :] = hh[8 * g:8 * g + 8]
                drain(side, share(n, g, ng))

        def mm2(c, side, n):
            cs = slice(c * CT, (c + 1) * CT)
            hid = asbf(jnp.concatenate([hid32[pl.ds(hid0 + t * MH, m // 2), :] for t in range(NT)], axis=1))
            o = jnp.dot(hid, asbf(w232[c]), preferred_element_type=jnp.float32)
            o = as32((o + b2[:, cs] + q_ref[rows, cs].astype(jnp.float32)).astype(bf))
            for g in range(ng):
                pc32[pl.ds(C_BASE + c * TS + h0 + 8 * g, 8), :] = o[8 * g:8 * g + 8]
                drain(side, share(n, g, ng))

        return ln, mm1, mm2

    def prep_pieces(j, oz):
        RB = 16
        k32, v32, f32v = (pc32.at[pl.ds(pl.multiple_of(c + j * TS + oz, 8), TS)] for c in (C_K, C_V, C_F))

        def prep_k(i):
            def run():
                s = [prm_ref[j, t:t + 1, :] for t in range(KS)]
                pk = []
                for p in range(8):
                    pk.extend(_unpack(k32[pl.ds(8 * RB * i + p, RB, stride=8), :]))
                if i == 0:
                    row = jax.lax.broadcasted_iota(jnp.int32, (RB, CT), 0)
                    pm = [jnp.where(row == 0, 0.0, pltpu.roll(pk[n], 1, 0)) for n in (13, 14, 15)]
                else:
                    pm = [_unpack(k32[pl.ds(8 * RB * i - 2, RB, stride=8), :])[1],
                          *_unpack(k32[pl.ds(8 * RB * i - 1, RB, stride=8), :])]
                pk = pm + pk
                for p in range(8):
                    vv = _unpack(v32[pl.ds(8 * RB * i + p, RB, stride=8), :])
                    for e in range(2):
                        n2 = 2 * p + e
                        ksh = pk[n2 + 3] * s[0] + pk[n2 + 2] * s[1] + pk[n2 + 1] * s[2] + pk[n2] * s[3]
                        r32[0, n2, pl.ds(RB // 2 * i, RB // 2), :] = as32((ksh * vv[e]).astype(bf))
            return run

        def prep_t(m):
            def run():
                t_ref[m * CT:(m + 1) * CT, :] = asbf(f32v[pl.ds(m * CT // 2, CT // 2), :]).astype(jnp.float32).T
            return run

        def prep_f(n2):
            def run():
                ft = t_ref[pl.ds(n2, N1, stride=16), :]
                if n2 == 0:
                    row = jax.lax.broadcasted_iota(jnp.int32, (N1, CT), 0)
                    ft = ft + jnp.where(row == 0, prm_ref[j, KS:KS + 1, :], 0.0)
                r32[1, n2] = as32(ft.astype(bf))
            return run

        return ([prep_t(m) for m in range(S // CT)], [prep_f(n) for n in range(N2)],
                [prep_k(i) for i in range(N1 // RB)])

    def conv_pieces(j, oz):
        def arow(z, n, r):
            return B_A + (z * N2 + n) * 2 * N1 + 16 * r

        def fwd(b):
            for z in range(2):
                x = [jnp.dot(asbf(g32[4 * a + b]), asbf(r32[z, 4 * a + b]), preferred_element_type=jnp.float32)
                     for a in range(4)]
                for r in range(N1 // 8):
                    y = _r4([(x[a][16 * r:16 * r + 8], x[a][16 * r + 8:16 * r + 16]) for a in range(4)], 1)
                    for c in range(4):
                        yr, yi = _tw(y[c], b, c, 1)
                        pb32[pl.ds(arow(z, 4 * c + b, r), 8), :] = as32(yr)
                        pb32[pl.ds(arow(z, 4 * c + b, r) + 8, 8), :] = as32(yi)

        def mid(c, r):
            def run():
                zx, zk = (_r4([(asf(pb32[pl.ds(oz + arow(z, 4 * c + b, r), 8), :]),
                                asf(pb32[pl.ds(oz + arow(z, 4 * c + b, r) + 8, 8), :])) for b in range(4)], 1,
                              rot2=(c == 2)) for z in range(2))
                yy = [(xr * kr - xi * ki, xr * ki + xi * kr) for (xr, xi), (kr, ki) in zip(zx, zk)]
                u = _r4(yy, -1)
                for b in range(4):
                    ur, ui = _tw(u[b], b, c, -1)
                    b_ref[4 * b + c, 16 * r:16 * r + 8, :] = ur
                    b_ref[4 * b + c, 16 * r + 8:16 * r + 16, :] = ui
            return run

        def inv(b):
            o = [[] for _ in range(4)]
            for r in range(N1 // 8):
                z = _r4([(b_ref[4 * b + c, pl.ds(oz + 16 * r, 8), :], b_ref[4 * b + c, pl.ds(oz + 16 * r + 8, 8), :])
                         for c in range(4)], -1, rot2=(b == 2))
                for a in range(4):
                    o[a].append(jnp.concatenate(z[a], axis=0).astype(bf))
            for a in range(4):
                y_ref[j, 4 * a + b] = jnp.dot(asbf(h32[4 * a + b]), jnp.concatenate(o[a], axis=0),
                                              preferred_element_type=jnp.float32)

        return fwd, [mid(c, r) for c in range(4) for r in range(N1 // 8)], inv

    def combine(j, a, n, p, oz):
        def run():
            sl = pl.ds(8 * a + p, n, stride=8)
            b_lo, b_hi = _unpack(pc32.at[pl.ds(oz + C_BASE + j * TS, TS)][sl, :])
            x_lo, x_hi = _unpack(xn32[j, sl, :])
            o_lo = b_lo + x_lo * y_ref[j, 2 * p, a:a + n, :]
            o_hi = b_hi + x_hi * y_ref[j, 2 * p + 1, a:a + n, :]
            o32[j, sl, :] = pltpu.pack_elementwise([o_lo, o_hi], packed_dtype=bf)
        return run

    ln, mm1, mm2 = mlp_pieces(0, MP, pb32, B_HID)
    c_q0.wait()
    for c in c_w1[1]:
        c.start()
    ln()
    for i, ts in enumerate((range(0, 2), range(2, 6), range(6, NT))):
        for c in c_w1[i]:
            c.wait()
        if i == 0:
            for c in c_w1[2]:
                c.start()
        elif i == 1:
            for c in c_w2:
                c.start()
        else:
            kvf_start(0)
        for t in ts:
            mm1(t, [], 0)
    for c in c_w2:
        c.wait()
    q_copy(0).start()
    c_g.start()
    mm2(0, [], 0)
    mm2(1, [], 0)
    kvf_wait(0)
    c_h.start()
    q_copy(1).start()
    pt, pf, pk = prep_pieces(0, 0)
    drain(pt, 16)
    drain(pk, 3)
    side = pf + pk
    for c, n in ((2, 19), (3, 2), (4, 0)):
        mm2(c, side, n)
    q_copy(0).wait()
    c_g.wait()
    kvf_start(1)
    mlp_pieces(MP, MM, pb32, B_HID)[0]()
    for b in range(4):
        conv_pieces(0, 0)[0](b)
    c_h.wait()
    oz = ((g32[0, 0, 0] ^ jnp.uint32(int(_G[0, 0, 0]))) << 3).astype(jnp.int32)

    def body(j, oz):
        kvf_wait(j + 1)
        q_copy(j + 1).wait()

        @pl.when(j + 2 < NCT)
        def _():
            kvf_start(j + 2)
            q_copy(j + 2).start()

        oz = pl.multiple_of(oz, 8)
        r0 = pl.multiple_of(MP + j * MM, 16)
        _, mm1, mm2 = mlp_pieces(r0, MM, pb32, B_HID)
        _, side, inv = conv_pieces(j, oz)
        for t, n in enumerate((6, 5, 5, 5, 5, 5, 5, 5, 5, 5, 5, 5, 3, 0)):
            mm1(t, side, n)
        pt, pf, pk = prep_pieces(j + 1, oz)
        fwd = conv_pieces(j + 1, oz)[0]
        drain(pt, 16)
        side = pk[:4] + pf + pk[4:]
        for c, n in enumerate((4, 18, 2, 0, 0)):
            if c < 4:
                inv(c)
            mm2(c, side, n)
            if c == 2:
                mlp_pieces(pl.multiple_of(r0 + MM, 16), MM, pb32, B_HID)[0]()
        for b in range(4):
            fwd(b)
        return oz

    oz = pl.multiple_of(jax.lax.fori_loop(0, NCT - 1, body, oz), 8)

    _, mm1, _ = mlp_pieces(S - ME, ME, pb32, B_HID)
    _, side, inv = conv_pieces(NCT - 1, oz)
    for t, n in enumerate((6, 5, 5, 5, 5, 5, 5, 5, 5, 5, 5, 5, 3, 0)):
        mm1(t, side, n)
    mm2 = mlp_pieces(S - ME, ME, pb32, B_HID)[2]
    na = (S - ME) // 16
    cuts = list(range(0, na, 16)) + [na]
    c_out = [copy(o_ref.at[j, 0:S - ME], o_hbm.at[0:S - ME, j * CT:(j + 1) * CT]) for j in range(NCT)]
    for c in range(NCT):
        if c < 4:
            inv(c)
        side = []
        if c < 4:
            for j in ((0, 1), (2, 3), (), (4,))[c]:
                side += [combine(j, a0, a1 - a0, p, oz) for a0, a1 in zip(cuts[:-1], cuts[1:]) for p in range(8)]
        if c == 0:
            drain(side, 16)
        mm2(c, side, len(side))
        if c < 4:
            for j in ((0, 1), (2, 3), (), (4,))[c]:
                c_out[j].start()
    for j in range(NCT):
        for p in range(8):
            combine(j, na, ME // 16, p, 0)()
    c_last = [copy(o_ref.at[j, S - ME:S], o_hbm.at[S - ME:S, j * CT:(j + 1) * CT]) for j in range(NCT)]
    for c in c_last:
        c.start()
    for c in c_out + c_last:
        c.wait()


@jax.jit
def pallas_parallel_sum__ssm_conv_h3__dense_activation_gelu__prompt_kernel(
        A_q, A_k, A_v, A_shift_k, A_ssm_k, A_ssm_D, B_x, B_w1, B_b1, B_w2, B_b2):
    hb = pl.BlockSpec(memory_space=pltpu.HBM)
    u32, f32, bf = jnp.uint32, jnp.float32, jnp.bfloat16
    mh = max(MP, MM, ME)
    out = pl.pallas_call(
        _kernel,
        out_shape=jax.ShapeDtypeStruct((S, D), A_q.dtype),
        in_specs=[hb] * 12,
        out_specs=hb,
        scratch_shapes=[
            pltpu.VMEM((S, D), bf),
            pltpu.VMEM((2 * C_ROWS + 16, CT), bf),
            pltpu.VMEM((NCT, FP, CT), bf),
            pltpu.VMEM((NCT, FP, CT), bf),
            pltpu.VMEM((N2, N1, N1), u32),
            pltpu.VMEM((N2, N1 // 2, 2 * N1), u32),
            pltpu.VMEM((NCT, S, CT), bf),
            pltpu.VMEM((NCT, S // 2, CT), u32),
            pltpu.VMEM((B_ROWS + 8, CT), u32),
            pltpu.VMEM((2, N2, N1 // 2, CT), u32),
            pltpu.VMEM((N2, 2 * N1 + 8, CT), f32),
            pltpu.VMEM((S, CT), f32),
            pltpu.VMEM((KS, D), bf),
            pltpu.VMEM((D,), bf),
            pltpu.VMEM((F,), bf),
            pltpu.VMEM((D,), bf),
            pltpu.VMEM((NCT, 8, CT), f32),
            pltpu.VMEM((NCT, N2, N1, CT), f32),
            pltpu.SemaphoreType.DMA((80,)),
        ],
        compiler_params=pltpu.CompilerParams(vmem_limit_bytes=100 * 1024 * 1024),
    )(A_q.reshape(S, D), A_k.reshape(S, D), A_v.reshape(S, D), A_shift_k.T, A_ssm_k, A_ssm_D,
      B_w1.T, B_b1, B_w2, B_b2, jnp.asarray(_G), jnp.asarray(_H))
    return out.reshape(1, S, D)
```

```python
import functools
import numpy as np
import jax
import jax.numpy as jnp
import jax.experimental.pallas as pl
import jax.experimental.pallas.tpu as pltpu

S, D, F, KS = 2048, 640, 1728, 4
FP = 1792
N1, N2 = 128, 16
CT = 128
NCT = D // CT
MP, MM = 448, 320
ME = MM
MID_PLAN = (6, 5, 5, 5, 5, 5, 5, 5, 5, 5, 5, 4, 4, 0)
FC = 256
MH = max(MP, MM, ME) // 2
NT = FP // CT
B_HID = 0
B_A = NT * MH
B_ROWS = B_A + 2 * N2 * 2 * N1
TS = S // 2
C_K, C_V, C_BASE = 0, NCT * TS, 2 * NCT * TS
C_ROWS = 3 * NCT * TS
assert MP + (NCT - 1) * MM + ME == S


def _dft_consts():
    n1 = np.arange(N1)
    k1 = np.arange(N1)
    g = np.zeros((N2, 2 * N1, N1), np.float64)
    for n2 in range(N2):
        t = N2 * n1 + n2
        ph = np.pi * t[None, :] / (2 * S) - 2 * np.pi * ((t[None, :] * k1[:, None]) % S) / S
        g[n2, :N1] = np.cos(ph)
        g[n2, N1:] = np.sin(ph)
    g = g.reshape(N2, 2, N1 // 8, 8, N1).transpose(0, 2, 1, 3, 4).reshape(N2, 2 * N1, N1)
    h = np.transpose(g, (0, 2, 1)) / S

    def pack(m):
        u = np.ascontiguousarray(m).astype(jnp.bfloat16).view(np.uint16).astype(np.uint32)
        return u[:, 0::2, :] | (u[:, 1::2, :] << 16)

    return pack(g), pack(h)


_G, _H = _dft_consts()


def _cmul_const(re, im, e):
    e = e % 16
    if e == 0:
        return re, im
    c = float(np.cos(2 * np.pi * e / 16))
    s = float(-np.sin(2 * np.pi * e / 16))
    if e % 2 == 0:
        if c * s > 0:
            return (re - im) * c, (re + im) * c
        return (re + im) * c, (im - re) * c
    return re * c - im * s, re * s + im * c


def _r4(x, sign, rot2=False):
    (ar, ai), (br, bi), (cr, ci), (dr, di) = x
    if not rot2:
        t0r, t0i = ar + cr, ai + ci
        t1r, t1i = ar - cr, ai - ci
    elif sign > 0:
        t0r, t0i = ar + ci, ai - cr
        t1r, t1i = ar - ci, ai + cr
    else:
        t0r, t0i = ar - ci, ai + cr
        t1r, t1i = ar + ci, ai - cr
    t2r, t2i = br + dr, bi + di
    t3r, t3i = br - dr, bi - di
    y0 = (t0r + t2r, t0i + t2i)
    y2 = (t0r - t2r, t0i - t2i)
    ym = (t1r + t3i, t1i - t3r)
    yp = (t1r - t3i, t1i + t3r)
    if sign > 0:
        return [y0, ym, y2, yp]
    return [y0, yp, y2, ym]


def _tw(y, b, c, sign):
    return y if b * c == 4 else _cmul_const(*y, sign * b * c)


def _unpack(u):
    lo = pltpu.bitcast(u << 16, jnp.float32)
    hi = pltpu.bitcast(u & jnp.uint32(0xFFFF0000), jnp.float32)
    return lo, hi


def _gelu(h):
    c0 = float(np.sqrt(2 / np.pi))
    c1 = c0 * 0.044715
    u = h * (c0 + c1 * (h * h))
    hh = 0.5 * h
    return hh + hh * jnp.tanh(u)


def _kernel(q_hbm, k_hbm, v_hbm, sk_hbm, f_hbm, d_hbm, w1_hbm, b1_hbm, w2_hbm, b2_hbm, g_hbm, h_hbm,
            o_hbm,
            q_ref, pc_ref, f_ref, w1_ref, w2_ref, g32, h32, o_ref, xn32, pb32, r32, b_ref, t_ref,
            sk_ref, d_ref, b1_ref, b2_ref, prm_ref, y_ref, sems):
    bf = jnp.bfloat16
    u32 = jnp.uint32
    pc32, o32, w132, w232 = (r.bitcast(u32) for r in (pc_ref, o_ref, w1_ref, w2_ref))
    asf = lambda x: pltpu.bitcast(x, jnp.float32)
    asbf = lambda x: pltpu.bitcast(x, bf)
    as32 = lambda x: pltpu.bitcast(x, u32)

    nsem = [0]

    def copy(src, dst):
        c = pltpu.make_async_copy(src, dst, sems.at[nsem[0]])
        nsem[0] += 1
        return c

    c_q0 = copy(q_hbm.at[0:MP], q_ref.at[0:MP])
    c_small = [copy(sk_hbm, sk_ref), copy(d_hbm, d_ref), copy(b1_hbm, b1_ref), copy(b2_hbm, b2_ref)]
    c_w1 = [[copy(w1_hbm.at[f0:f1, c * CT:(c + 1) * CT], w1_ref.at[c, f0:f1]) for c in range(NCT)]
            for f0, f1 in ((0, FC), (FC, 3 * FC), (3 * FC, F))]
    c_w2 = [copy(w2_hbm.at[:, c * CT:(c + 1) * CT], w2_ref.at[c, 0:F]) for c in range(NCT)]
    c_g = copy(g_hbm, g32)
    c_h = copy(h_hbm, h32)
    c_kvf = [[copy(f_hbm.at[j * CT:(j + 1) * CT], f_ref.at[j]),
              copy(k_hbm.at[:, j * CT:(j + 1) * CT], pc_ref.at[2 * (C_K + j * TS):2 * (C_K + (j + 1) * TS)]),
              copy(v_hbm.at[:, j * CT:(j + 1) * CT], pc_ref.at[2 * (C_V + j * TS):2 * (C_V + (j + 1) * TS)])]
             for j in range(NCT)]
    c_q = [copy(q_hbm.at[r0:r1], q_ref.at[r0:r1]) for r0, r1 in ((MP, MP + MM), (MP + MM, MP + 2 * MM), (MP + 2 * MM, S))]

    def start(cs):
        for c in cs:
            c.start()

    def wait(cs):
        for c in cs:
            c.wait()

    for c in [c_q0] + c_w1[0] + c_small + c_w1[1]:
        c.start()

    w1_ref[:, F:FP, :] = jnp.zeros((NCT, FP - F, CT), bf)
    w2_ref[:, F:FP, :] = jnp.zeros((NCT, FP - F, CT), bf)
    for c in c_small:
        c.wait()
    b1 = b1_ref[...].astype(jnp.float32).reshape(1, F)
    b1 = jnp.concatenate([b1, jnp.zeros((1, FP - F), jnp.float32)], axis=1)
    b2 = b2_ref[...].astype(jnp.float32).reshape(1, D)
    dd = d_ref[...].astype(jnp.float32).reshape(1, D)
    skt = sk_ref[...].astype(jnp.float32)
    for j in range(NCT):
        prm_ref[j, 0:KS, :] = skt[:, j * CT:(j + 1) * CT]
        prm_ref[j, KS:KS + 1, :] = dd[:, j * CT:(j + 1) * CT]

    def drain(q, n):
        toks = []
        for _ in range(n):
            if q:
                toks.append(q.pop(0)())
        return toks

    def tie(x, toks, oz):
        if not toks:
            return x
        t = functools.reduce(jnp.bitwise_or, [as32(z) for z in toks]) & oz.astype(u32)
        return jnp.concatenate([x[0:8] | t, x[8:]], axis=0)

    def share(n, i, parts):
        return (i + 1) * n // parts - i * n // parts

    def mlp_pieces(r0, m, hid32, hid0):
        rows = pl.ds(r0, m)
        h0 = r0 // 2 if isinstance(r0, int) else pl.multiple_of(r0 // 2, 8)
        ng = m // 16

        def ln():
            x = q_ref[rows, :].astype(jnp.float32)
            mu = jnp.mean(x, axis=-1, keepdims=True)
            xc = x - mu
            var = jnp.mean(xc * xc, axis=-1, keepdims=True)
            xn = as32((xc * jax.lax.rsqrt(var + 1e-5)).astype(bf))
            for c in range(NCT):
                xn32[c, pl.ds(h0, m // 2), :] = xn[:, c * CT:(c + 1) * CT]

        def mm1(t, side, n, toks=(), oz=None):
            xn = [xn32[c, pl.ds(h0, m // 2), :] for c in range(NCT)]
            xn = asbf(jnp.concatenate([tie(xn[0], toks, oz)] + xn[1:], axis=1))
            w = asbf(jnp.concatenate([w132[c, t * CT // 2:(t + 1) * CT // 2, :] for c in range(NCT)], axis=1))
            hh = jax.lax.dot_general(xn, w, (((1,), (1,)), ((), ())),
                                     preferred_element_type=jnp.float32) + b1[:, t * CT:(t + 1) * CT]
            hh = as32(_gelu(hh).astype(bf))
            out = []
            for g in range(ng):
                hid32[pl.ds(hid0 + t * MH + 8 * g, 8), :] = hh[8 * g:8 * g + 8]
                out += drain(side, share(n, g, ng))
            return out

        def mm2(c, side, n, hook=None, toks=(), oz=None):
            cs = slice(c * CT, (c + 1) * CT)
            hid, w = [], []
            for t in range(NT):
                if t == NT - 2 and hook is not None:
                    hook()
                hid.append(hid32[pl.ds(hid0 + t * MH, m // 2), :])
                w.append(w232[c, t * CT // 2:(t + 1) * CT // 2, :])
            hid[0] = tie(hid[0], toks, oz)
            o = jnp.dot(asbf(jnp.concatenate(hid, axis=1)), asbf(jnp.concatenate(w, axis=0)),
                        preferred_element_type=jnp.float32)
            o = as32((o + b2[:, cs] + q_ref[rows, cs].astype(jnp.float32)).astype(bf))
            out = []
            for g in range(ng):
                pc32[pl.ds(C_BASE + c * TS + h0 + 8 * g, 8), :] = o[8 * g:8 * g + 8]
                out += drain(side, share(n, g, ng))
            return out

        return ln, mm1, mm2

    def prep_pieces(j, oz):
        RB = 16
        k32, v32 = (pc32.at[pl.ds(pl.multiple_of(c + j * TS + oz, 8), TS)] for c in (C_K, C_V))

        def prep_k(i):
            def run():
                s = [prm_ref[j, t:t + 1, :] for t in range(KS)]
                pk = []
                for p in range(8):
                    pk.extend(_unpack(k32[pl.ds(8 * RB * i + p, RB, stride=8), :]))
                if i == 0:
                    row = jax.lax.broadcasted_iota(jnp.int32, (RB, CT), 0)
                    pm = [jnp.where(row == 0, 0.0, pltpu.roll(pk[n], 1, 0)) for n in (13, 14, 15)]
                else:
                    pm = [_unpack(k32[pl.ds(8 * RB * i - 2, RB, stride=8), :])[1],
                          *_unpack(k32[pl.ds(8 * RB * i - 1, RB, stride=8), :])]
                pk = pm + pk
                for p in range(8):
                    vv = _unpack(v32[pl.ds(8 * RB * i + p, RB, stride=8), :])
                    for e in range(2):
                        n2 = 2 * p + e
                        ksh = pk[n2 + 3] * s[0] + pk[n2 + 2] * s[1] + pk[n2 + 1] * s[2] + pk[n2] * s[3]
                        res = as32((ksh * vv[e]).astype(bf))
                        r32[0, n2, pl.ds(RB // 2 * i, RB // 2), :] = res
                        tok = res if n2 == 0 else tok | res
                return tok
            return run

        def prep_t(m):
            def run():
                ft = f_ref[j, :, m * CT:(m + 1) * CT].astype(jnp.float32).T
                t_ref[m * CT:(m + 1) * CT, :] = ft
                return ft[CT - 8:]
            return run

        def prep_f(n2):
            def run():
                ft = t_ref[pl.ds(n2, N1, stride=16), :]
                if n2 == 0:
                    row = jax.lax.broadcasted_iota(jnp.int32, (N1, CT), 0)
                    ft = ft + jnp.where(row == 0, prm_ref[j, KS:KS + 1, :], 0.0)
                res = as32(ft.astype(bf))
                r32[1, n2] = res
                return functools.reduce(jnp.bitwise_or, [res[i:i + 8] for i in range(0, N1 // 2, 8)])
            return run

        return ([prep_t(m) for m in range(S // CT)], [prep_f(n) for n in range(N2)],
                [prep_k(i) for i in range(N1 // RB)])

    def conv_pieces(j, oz):
        def arow(z, n, r):
            return B_A + (z * N2 + n) * 2 * N1 + 16 * r

        def fwd(b):
            for z in range(2):
                x = [jnp.dot(asbf(g32[4 * a + b]), asbf(r32[z, 4 * a + b]), preferred_element_type=jnp.float32)
                     for a in range(4)]
                for r in range(N1 // 8):
                    y = _r4([(x[a][16 * r:16 * r + 8], x[a][16 * r + 8:16 * r + 16]) for a in range(4)], 1)
                    for c in range(4):
                        yr, yi = _tw(y[c], b, c, 1)
                        pb32[pl.ds(arow(z, 4 * c + b, r), 8), :] = as32(yr)
                        pb32[pl.ds(arow(z, 4 * c + b, r) + 8, 8), :] = as32(yi)

        def mid(c, r):
            def run():
                zx, zk = (_r4([(asf(pb32[pl.ds(oz + arow(z, 4 * c + b, r), 8), :]),
                                asf(pb32[pl.ds(oz + arow(z, 4 * c + b, r) + 8, 8), :])) for b in range(4)], 1,
                              rot2=(c == 2)) for z in range(2))
                yy = [(xr * kr - xi * ki, xr * ki + xi * kr) for (xr, xi), (kr, ki) in zip(zx, zk)]
                u = _r4(yy, -1)
                for b in range(4):
                    ur, ui = _tw(u[b], b, c, -1)
                    b_ref[4 * b + c, 16 * r:16 * r + 8, :] = ur
                    b_ref[4 * b + c, 16 * r + 8:16 * r + 16, :] = ui
                return ui
            return run

        def inv(b, side=(), n=0):
            o = [[] for _ in range(4)]
            for r in range(N1 // 8):
                z = _r4([(b_ref[4 * b + c, pl.ds(oz + 16 * r, 8), :], b_ref[4 * b + c, pl.ds(oz + 16 * r + 8, 8), :])
                         for c in range(4)], -1, rot2=(b == 2))
                for a in range(4):
                    o[a].append(jnp.concatenate(z[a], axis=0).astype(bf))
            for a in range(4):
                o[a] = jnp.dot(asbf(h32[4 * a + b]), jnp.concatenate(o[a], axis=0),
                               preferred_element_type=jnp.float32)
            for g in range(8):
                for a in range(4):
                    y_ref[j, 4 * a + b, 16 * g:16 * g + 16, :] = o[a][16 * g:16 * g + 16]
                drain(side, share(n, g, 8))

        return fwd, [mid(c, r) for c in range(4) for r in range(N1 // 8)], inv

    def combine(j, a, n, p, oz):
        def run():
            sl = pl.ds(8 * a + p, n, stride=8)
            b_lo, b_hi = _unpack(pc32.at[pl.ds(oz + C_BASE + j * TS, TS)][sl, :])
            x_lo, x_hi = _unpack(xn32[j, sl, :])
            o_lo = b_lo + x_lo * y_ref[j, 2 * p, pl.ds(oz + a, n), :]
            o_hi = b_hi + x_hi * y_ref[j, 2 * p + 1, pl.ds(oz + a, n), :]
            o32[j, sl, :] = pltpu.pack_elementwise([o_lo, o_hi], packed_dtype=bf)
        return run

    def first_half(j, r0, oz):
        side = conv_pieces(j, oz)[1]
        mm1 = mlp_pieces(r0, MM, pb32, B_HID)[1]
        for t, n in enumerate(MID_PLAN):
            mm1(t, side, n)

    ln, mm1, mm2 = mlp_pieces(0, MP, pb32, B_HID)
    c_q0.wait()
    start(c_w1[2])
    ln()
    for i, ts in enumerate((range(0, 2), range(2, 6), range(6, NT))):
        wait(c_w1[i])
        start((c_w2, c_kvf[0], [c_q[0], c_g])[i])
        for t in ts:
            mm1(t, [], 0)
    wait(c_w2)
    mm2(0, [], 0)
    mm2(1, [], 0)
    mm2(2, [], 0)
    wait(c_kvf[0] + [c_q[0], c_g])
    start([c_h, c_q[1]] + c_kvf[1])
    oz = pl.multiple_of(((g32[0, 0, 0] ^ jnp.uint32(int(_G[0, 0, 0]))) << 3).astype(jnp.int32), 8)
    pt, pf, pk = prep_pieces(0, oz)
    drain(pt + pk + pf, 1 << 20)
    mlp_pieces(MP, MM, pb32, B_HID)[0]()
    mm2(3, [], 0)
    for b in range(4):
        conv_pieces(0, oz)[0](b)
    mm2(4, [], 0)
    wait([c_h, c_q[1]] + c_kvf[1])
    start(sum(c_kvf[2:], []) + [c_q[2]])

    def body(j, oz):
        pl.when(j == 1)(lambda: wait(sum(c_kvf[2:], []) + [c_q[2]]))
        oz = pl.multiple_of(oz, 8)
        r0 = pl.multiple_of(MP + j * MM, 16)
        r1 = pl.multiple_of(MP + (j + 1) * MM, 16)
        mm2 = mlp_pieces(r0, MM, pb32, B_HID)[2]
        inv = conv_pieces(j, oz)[2]
        fwd = conv_pieces(j + 1, oz)[0]
        pt, pf, pk = prep_pieces(j + 1, oz)
        first_half(j, r0, oz)
        side = pt + pk[:4] + pf + pk[4:]
        mm2(0, side, 20)
        inv(0)
        mlp_pieces(r1, MM, pb32, B_HID)[0]()
        mm2(1, side, 20)
        inv(1)
        inv(2)
        mm2(2, [], 0)
        inv(3)
        mm2(3, [], 0)
        for b in range(4):
            fwd(b)
        mm2(4, [], 0)
        return oz

    oz = pl.multiple_of(jax.lax.fori_loop(0, NCT - 1, body, oz), 8)

    first_half(NCT - 1, S - ME, oz)
    inv = conv_pieces(NCT - 1, oz)[2]
    mm2 = mlp_pieces(S - ME, ME, pb32, B_HID)[2]
    na = (S - ME) // 16
    cuts = list(range(0, na, 16)) + [na]
    c_out = [copy(o_ref.at[j, 0:S - ME], o_hbm.at[0:S - ME, j * CT:(j + 1) * CT]) for j in range(NCT)]
    c_last = [copy(o_ref.at[j, S - ME:S], o_hbm.at[S - ME:S, j * CT:(j + 1) * CT]) for j in range(NCT)]

    def head(j):
        return [combine(j, a0, a1 - a0, p, oz) for a0, a1 in zip(cuts[:-1], cuts[1:]) for p in range(8)]

    side = head(0) + head(1)
    for b in range(4):
        inv(b, side, share(len(head(0)) * 2, b, 4))
    for c in range(NCT):
        side = head(c + 2) if c < 3 else []
        mm2(c, side, len(side), lambda: start((c_out[0:2] if c == 0 else c_out[c + 1:c + 2]) + c_last[max(c - 1, 0):c]))
        for p in range(8):
            combine(c, na, ME // 16, p, 0)()
    start(c_last[NCT - 1:])
    wait(c_out + c_last)


@jax.jit
def pallas_parallel_sum__ssm_conv_h3__dense_activation_gelu__prompt_kernel(
        A_q, A_k, A_v, A_shift_k, A_ssm_k, A_ssm_D, B_x, B_w1, B_b1, B_w2, B_b2):
    hb = pl.BlockSpec(memory_space=pltpu.HBM)
    u32, f32, bf = jnp.uint32, jnp.float32, jnp.bfloat16
    mh = max(MP, MM, ME)
    out = pl.pallas_call(
        _kernel,
        out_shape=jax.ShapeDtypeStruct((S, D), A_q.dtype),
        in_specs=[hb] * 12,
        out_specs=hb,
        scratch_shapes=[
            pltpu.VMEM((S, D), bf),
            pltpu.VMEM((2 * C_ROWS + 16, CT), bf),
            pltpu.VMEM((NCT, CT, S), bf),
            pltpu.VMEM((NCT, FP, CT), bf),
            pltpu.VMEM((NCT, FP, CT), bf),
            pltpu.VMEM((N2, N1, N1), u32),
            pltpu.VMEM((N2, N1 // 2, 2 * N1), u32),
            pltpu.VMEM((NCT, S, CT), bf),
            pltpu.VMEM((NCT, S // 2, CT), u32),
            pltpu.VMEM((B_ROWS + 8, CT), u32),
            pltpu.VMEM((2, N2, N1 // 2, CT), u32),
            pltpu.VMEM((N2, 2 * N1 + 8, CT), f32),
            pltpu.VMEM((S, CT), f32),
            pltpu.VMEM((KS, D), bf),
            pltpu.VMEM((D,), bf),
            pltpu.VMEM((F,), bf),
            pltpu.VMEM((D,), bf),
            pltpu.VMEM((NCT, 8, CT), f32),
            pltpu.VMEM((NCT, N2, N1 + 8, CT), f32),
            pltpu.SemaphoreType.DMA((80,)),
        ],
        compiler_params=pltpu.CompilerParams(vmem_limit_bytes=100 * 1024 * 1024),
    )(A_q.reshape(S, D), A_k.reshape(S, D), A_v.reshape(S, D), A_shift_k.T, A_ssm_k, A_ssm_D,
      B_w1.T, B_b1, B_w2, B_b2, jnp.asarray(_G), jnp.asarray(_H))
    return out.reshape(1, S, D)
```

```python
import functools
import numpy as np
import jax
import jax.numpy as jnp
import jax.experimental.pallas as pl
import jax.experimental.pallas.tpu as pltpu

S, D, F, KS = 2048, 640, 1728, 4
FP = 1792
N1, N2 = 128, 16
CT = 128
NCT = D // CT
MP, MM = 448, 320
ME = MM
MID_PLAN = (7, 6, 6, 5, 5, 5, 5, 5, 5, 5, 5, 5, 4, 0)
FC = 256
MH = max(MP, MM, ME) // 2
NT = FP // CT
B_HID = 0
B_A = NT * MH
B_ROWS = B_A + 2 * N2 * 2 * N1
TS = S // 2
C_K, C_V, C_BASE, C_Q = (i * NCT * TS for i in range(4))
C_TIE = 4 * NCT * TS
C_ROWS = C_TIE + 8
assert MP + (NCT - 1) * MM + ME == S


def _dft_consts():
    n1 = np.arange(N1)
    k1 = np.arange(N1)
    g = np.zeros((N2, 2 * N1, N1), np.float64)
    for n2 in range(N2):
        t = N2 * n1 + n2
        ph = np.pi * t[None, :] / (2 * S) - 2 * np.pi * ((t[None, :] * k1[:, None]) % S) / S
        g[n2, :N1] = np.cos(ph)
        g[n2, N1:] = np.sin(ph)
    g = g.reshape(N2, 2, N1 // 8, 8, N1).transpose(0, 2, 1, 3, 4).reshape(N2, 2 * N1, N1)
    h = np.transpose(g, (0, 2, 1)) / S
    h = h.reshape(N2, N1, 2 * N1 // 16, 2, 8).transpose(0, 1, 2, 4, 3).reshape(N2, N1, 2 * N1)
    g = g.reshape(N2, 2 * N1, N1 // 16, 2, 8).transpose(0, 1, 2, 4, 3).reshape(N2, 2 * N1, N1)

    def pack(m):
        u = np.ascontiguousarray(m).astype(jnp.bfloat16).view(np.uint16).astype(np.uint32)
        return u[:, 0::2, :] | (u[:, 1::2, :] << 16)

    return pack(g), pack(h)


_G, _H = _dft_consts()


def _cmul_const(re, im, e):
    e = e % 16
    if e == 0:
        return re, im
    c = float(np.cos(2 * np.pi * e / 16))
    s = float(-np.sin(2 * np.pi * e / 16))
    if e % 2 == 0:
        if c * s > 0:
            return (re - im) * c, (re + im) * c
        return (re + im) * c, (im - re) * c
    return re * c - im * s, re * s + im * c


def _r4(x, sign, rot2=False):
    (ar, ai), (br, bi), (cr, ci), (dr, di) = x
    if not rot2:
        t0r, t0i = ar + cr, ai + ci
        t1r, t1i = ar - cr, ai - ci
    elif sign > 0:
        t0r, t0i = ar + ci, ai - cr
        t1r, t1i = ar - ci, ai + cr
    else:
        t0r, t0i = ar - ci, ai + cr
        t1r, t1i = ar + ci, ai - cr
    t2r, t2i = br + dr, bi + di
    t3r, t3i = br - dr, bi - di
    y0 = (t0r + t2r, t0i + t2i)
    y2 = (t0r - t2r, t0i - t2i)
    ym = (t1r + t3i, t1i - t3r)
    yp = (t1r - t3i, t1i + t3r)
    if sign > 0:
        return [y0, ym, y2, yp]
    return [y0, yp, y2, ym]


def _tw(y, b, c, sign):
    return y if b * c == 4 else _cmul_const(*y, sign * b * c)


def _unpack(u):
    lo = pltpu.bitcast(u << 16, jnp.float32)
    hi = pltpu.bitcast(u & jnp.uint32(0xFFFF0000), jnp.float32)
    return lo, hi


def _pack(x):
    return pltpu.pack_elementwise([x[0:8], x[8:16]], packed_dtype=jnp.bfloat16)


def _gelu(h):
    c0 = float(np.sqrt(2 / np.pi))
    c1 = c0 * 0.044715
    u = h * (c0 + c1 * (h * h))
    hh = 0.5 * h
    return hh + hh * jnp.tanh(u)


def _kernel(q_hbm, k_hbm, v_hbm, sk_hbm, f_hbm, d_hbm, w1_hbm, b1_hbm, w2_hbm, b2_hbm, g_hbm, h_hbm,
            o_hbm,
            pc_ref, f_ref, w1_ref, w2_ref, g32, h32, o_ref, xn32, pb32, r32, b32, w_ref, t_ref,
            sk_ref, d_ref, b1_ref, b2_ref, prm_ref, y_ref, sems):
    bf = jnp.bfloat16
    u32 = jnp.uint32
    pc32, o32, w132, w232 = (r.bitcast(u32) for r in (pc_ref, o_ref, w1_ref, w2_ref))
    asf = lambda x: pltpu.bitcast(x, jnp.float32)
    asbf = lambda x: pltpu.bitcast(x, bf)
    as32 = lambda x: pltpu.bitcast(x, u32)

    nsem = [0]

    def copy(src, dst):
        c = pltpu.make_async_copy(src, dst, sems.at[nsem[0]])
        nsem[0] += 1
        return c

    def q_copies(r0, r1):
        return [copy(q_hbm.at[r0:r1, c * CT:(c + 1) * CT], pc_ref.at[2 * (C_Q + c * TS) + r0:2 * (C_Q + c * TS) + r1])
                for c in range(NCT)]

    c_q0 = q_copies(0, MP)
    c_small = [copy(sk_hbm, sk_ref), copy(d_hbm, d_ref), copy(b1_hbm, b1_ref), copy(b2_hbm, b2_ref)]
    c_w1 = [[copy(w1_hbm.at[f0:f1, c * CT:(c + 1) * CT], w1_ref.at[c, f0:f1]) for c in range(NCT)]
            for f0, f1 in ((0, FC), (FC, 3 * FC), (3 * FC, F))]
    c_w2 = [copy(w2_hbm.at[:, c * CT:(c + 1) * CT], w2_ref.at[c, 0:F]) for c in range(NCT)]
    c_g = copy(g_hbm, g32)
    c_h0 = copy(h_hbm.at[0], h32.at[0])
    c_h = copy(h_hbm.at[1:N2], h32.at[1:N2])
    c_kvf = [[copy(f_hbm.at[j * CT:(j + 1) * CT], f_ref.at[j]),
              copy(k_hbm.at[:, j * CT:(j + 1) * CT], pc_ref.at[2 * (C_K + j * TS):2 * (C_K + (j + 1) * TS)]),
              copy(v_hbm.at[:, j * CT:(j + 1) * CT], pc_ref.at[2 * (C_V + j * TS):2 * (C_V + (j + 1) * TS)])]
             for j in range(NCT)]
    c_q = [q_copies(r0, r1) for r0, r1 in ((MP, MP + MM), (MP + MM, MP + 2 * MM), (MP + 2 * MM, S))]

    def start(cs):
        for c in cs:
            c.start()

    def wait(cs):
        for c in cs:
            c.wait()

    for c in c_q0 + c_w1[0] + c_small + c_w1[1]:
        c.start()

    w1_ref[:, F:FP, :] = jnp.zeros((NCT, FP - F, CT), bf)
    w2_ref[:, F:FP, :] = jnp.zeros((NCT, FP - F, CT), bf)
    for c in c_small:
        c.wait()
    b1 = b1_ref[...].astype(jnp.float32).reshape(1, F)
    b1 = jnp.concatenate([b1, jnp.zeros((1, FP - F), jnp.float32)], axis=1)
    b2 = b2_ref[...].astype(jnp.float32).reshape(1, D)
    dd = d_ref[...].astype(jnp.float32).reshape(1, D)
    skt = sk_ref[...].astype(jnp.float32)
    for j in range(NCT):
        prm_ref[j, 0:KS, :] = skt[:, j * CT:(j + 1) * CT]
        prm_ref[j, KS:KS + 1, :] = dd[:, j * CT:(j + 1) * CT]

    def drain(q, n):
        toks = []
        for _ in range(n):
            if q:
                toks.append(q.pop(0)())
        return toks

    def tie(x, toks, oz):
        if not toks:
            return x
        t = functools.reduce(jnp.bitwise_or, [as32(z) for z in toks]) & oz.astype(u32)
        return x | t

    def share(n, i, parts):
        return -(-(i + 1) * n // parts) + (-i * n // parts)

    def mlp_pieces(r0, m, hid32, hid0):
        h0 = r0 // 2 if isinstance(r0, int) else pl.multiple_of(r0 // 2, 8)
        ng = m // 16

        def resid(c, g):
            x = asbf(pc32[pl.ds(C_Q + c * TS + h0 + 8 * g, 8), :]).astype(jnp.float32)
            return asbf(_pack(x)).astype(jnp.float32)

        def ln_rows(h, n):
            def run():
                u = jnp.concatenate([pc32[pl.ds(C_Q + c * TS + h, n), :] for c in range(NCT)], axis=1)
                x = jnp.concatenate(_unpack(u), axis=0)
                mu = jnp.mean(x, axis=-1, keepdims=True)
                xc = x - mu
                var = jnp.mean(xc * xc, axis=-1, keepdims=True)
                xn = xc * jax.lax.rsqrt(var + 1e-5)
                xn = pltpu.pack_elementwise([xn[0:n], xn[n:2 * n]], packed_dtype=bf)
                for c in range(NCT):
                    xn32[c, pl.ds(h, n), :] = xn[:, c * CT:(c + 1) * CT]
            return run

        ln = [ln_rows(h0 + 8 * g, 8 * min(2, ng - g)) for g in range(0, ng, 2)]

        def mm1(t, side, n, side_c=(), n_c=0, hook=None):
            xn = [xn32[c, pl.ds(h0, m // 2), :] for c in range(NCT)]
            xn = asbf(jnp.concatenate(xn, axis=1))
            w = asbf(jnp.concatenate([w132[c, t * CT // 2:(t + 1) * CT // 2, :] for c in range(NCT)], axis=1))
            if hook is not None:
                hook()
            hh = jax.lax.dot_general(xn, w, (((1,), (1,)), ((), ())),
                                     preferred_element_type=jnp.float32) + b1[:, t * CT:(t + 1) * CT]
            hh = _gelu(hh)
            hh = [_pack(hh[16 * g:16 * g + 16]) for g in range(ng)]
            out = []
            for g in range(ng):
                hid32[pl.ds(hid0 + t * MH + 8 * g, 8), :] = hh[g]
                drain(side, share(n, g, ng))
                if share(n_c, g, ng):
                    pc32[C_TIE:C_TIE + 8, :] = hh[g]
                    drain(side_c, share(n_c, g, ng))

        def mm2(c, side, n, hook=None, toks=(), oz=None):
            cs = slice(c * CT, (c + 1) * CT)
            hid, w = [], []
            for t in range(NT):
                if t == NT - 2 and hook is not None:
                    hook()
                x = [hid32[pl.ds(hid0 + t * MH + 8 * g, 8), :] for g in range(ng)]
                x[0] = tie(x[0], dict(toks).get(t), oz)
                hid.append(jnp.concatenate([asbf(z) for z in x], axis=0))
                w.append(w232[c, t * CT // 2:(t + 1) * CT // 2, :])
            o = jnp.dot(jnp.concatenate(hid, axis=1), asbf(jnp.concatenate(w, axis=0)),
                        preferred_element_type=jnp.float32)
            o = o + b2[:, cs]
            out = []
            for g in range(ng):
                pc32[pl.ds(C_BASE + c * TS + h0 + 8 * g, 8), :] = _pack(o[16 * g:16 * g + 16] + resid(c, g))
                out += drain(side, share(n, g, ng))
            return out

        return ln, mm1, mm2

    def prep_pieces(j, oz):
        RB = 16
        k32, v32 = (pc32.at[pl.ds(pl.multiple_of(c + j * TS + oz, 8), TS)] for c in (C_K, C_V))

        def prep_k(i):
            def run():
                s = [prm_ref[j, t:t + 1, :] for t in range(KS)]
                memo = {}

                def pk(n2):
                    p = n2 // 2
                    if p not in memo:
                        if p < 0 and i == 0:
                            row = jax.lax.broadcasted_iota(jnp.int32, (RB, CT), 0)
                            memo[p] = [jnp.where(row == 0, 0.0, pltpu.roll(pk(n + N2), 1, 0)) for n in (2 * p, 2 * p + 1)]
                        else:
                            memo[p] = _unpack(k32[pl.ds(8 * RB * i + p, RB, stride=8), :])
                    return memo[p][n2 % 2]

                for p in range(8):
                    vv = _unpack(v32[pl.ds(8 * RB * i + p, RB, stride=8), :])
                    for e in range(2):
                        n2 = 2 * p + e
                        ksh = pk(n2 - 3) * s[3] + pk(n2 - 2) * s[2] + pk(n2 - 1) * s[1] + pk(n2) * s[0]
                        res = _pack(ksh * vv[e])
                        r32[0, n2, pl.ds(RB // 2 * i, RB // 2), :] = res
                        tok = res if n2 == 0 else tok | res
                return tok
            return run

        def prep_t(m):
            def run():
                ft = f_ref[j, :, m * CT:(m + 1) * CT].astype(jnp.float32).T
                t_ref[m * CT:(m + 1) * CT, :] = ft
                return ft[CT - 8:]
            return run

        def prep_f(n2):
            def run():
                ft = t_ref[pl.ds(n2, N1, stride=16), :]
                if n2 == 0:
                    row = jax.lax.broadcasted_iota(jnp.int32, (N1, CT), 0)
                    ft = ft + jnp.where(row == 0, prm_ref[j, KS:KS + 1, :], 0.0)
                for g in range(N1 // 16):
                    r32[1, n2, 8 * g:8 * g + 8, :] = _pack(ft[16 * g:16 * g + 16])
                return ft[N1 - 8:]
            return run

        return ([prep_t(m) for m in range(S // CT)], [prep_f(n) for n in range(N2)],
                [prep_k(i) for i in range(N1 // RB)])

    def conv_pieces(j, oz):
        def arow(z, n, r):
            return B_A + (z * N2 + n) * 2 * N1 + 16 * r

        def fwd(b):
            for z in range(2):
                x = [jnp.dot(asbf(g32[4 * a + b]), asbf(r32[z, 4 * a + b]), preferred_element_type=jnp.float32)
                     for a in range(4)]
                for r in range(N1 // 8):
                    y = _r4([(x[a][16 * r:16 * r + 8], x[a][16 * r + 8:16 * r + 16]) for a in range(4)], 1)
                    for c in range(4):
                        yr, yi = _tw(y[c], b, c, 1)
                        pb32[pl.ds(arow(z, 4 * c + b, r), 8), :] = as32(yr)
                        pb32[pl.ds(arow(z, 4 * c + b, r) + 8, 8), :] = as32(yi)

        def mid(c, r):
            zx, zk = (_r4([(asf(pb32[pl.ds(oz + arow(z, 4 * c + b, r), 8), :]),
                            asf(pb32[pl.ds(oz + arow(z, 4 * c + b, r) + 8, 8), :])) for b in range(4)], 1,
                          rot2=(c == 2)) for z in range(2))
            yy = [(xr * kr - xi * ki, xr * ki + xi * kr) for (xr, xi), (kr, ki) in zip(zx, zk)]
            u = _r4(yy, -1)
            for b in range(4):
                ur, ui = _tw(u[b], b, c, -1)
                w_ref[4 * b + c, 16 * r:16 * r + 8, :] = ur
                w_ref[4 * b + c, 16 * r + 8:16 * r + 16, :] = ui

        def last(b, r):
            z = _r4([(w_ref[4 * b + c, pl.ds(oz + 16 * r, 8), :], w_ref[4 * b + c, pl.ds(oz + 16 * r + 8, 8), :])
                     for c in range(4)], -1, rot2=(b == 2))
            for a in range(4):
                b32[4 * a + b, 8 * r:8 * r + 8, :] = pltpu.pack_elementwise(list(z[a]), packed_dtype=bf)

        def spectrum(i):
            def run():
                if i >= 4:
                    last(i % 4, i // 4 - 1)
                if i < 64:
                    mid(i % 4, i // 4)
            return run

        def inv(b, side=(), n=0):
            o = [jnp.dot(asbf(h32[4 * a + b]), asbf(b32[4 * a + b, pl.ds(oz, N1), :]),
                         preferred_element_type=jnp.float32) for a in range(4)]
            for g in range(8):
                for a in range(4):
                    y_ref[j, 4 * a + b, 16 * g:16 * g + 16, :] = o[a][16 * g:16 * g + 16]
                drain(side, share(n, g, 8))

        return fwd, [spectrum(i) for i in range(68)], inv

    def combine(j, a, n, u, oz):
        def run():
            e = 8 * (u // 2) + 2 * (u % 2)
            rows = lambda w: pl.ds(8 * a + w, n, stride=8)
            base = pc32.at[pl.ds(oz + C_BASE + j * TS, TS)]
            b0, b1 = (_unpack(base[rows(2 * (e % 8 + i) + e // 8), :]) for i in range(2))
            for z in range(2):
                n2 = e + 4 * z
                x_lo, x_hi = _unpack(xn32[j, rows(n2 // 2), :])
                o_lo = b0[z] + x_lo * y_ref[j, n2, pl.ds(oz + a, n), :]
                o_hi = b1[z] + x_hi * y_ref[j, n2 + 1, pl.ds(oz + a, n), :]
                o32[j, rows(n2 // 2), :] = pltpu.pack_elementwise([o_lo, o_hi], packed_dtype=bf)
        return run

    def first_half(j, r0, oz, side_c, plan_c, hook=None):
        side = conv_pieces(j, oz)[1]
        mm1 = mlp_pieces(r0, MM, pb32, B_HID)[1]
        for t, n in enumerate(MID_PLAN):
            mm1(t, side, n, side_c, plan_c[t], hook if t == NT - 1 else None)

    ln, mm1, mm2 = mlp_pieces(0, MP, pb32, B_HID)
    wait(c_q0)
    start(c_w1[2])
    drain(ln, 1 << 20)
    for i, ts in enumerate((range(0, 2), range(2, 6), range(6, NT))):
        wait(c_w1[i])
        start((c_w2[:2] + c_kvf[0][:1], c_kvf[0][1:] + [c_h0], c_q[0] + c_w2[2:4])[i])
        for t in ts:
            mm1(t, [], 0)
    wait(c_w2[:2] + c_kvf[0] + [c_h0])
    start([c_g] + c_w2[4:])
    oz = pl.multiple_of(((h32[0, 0, 0] ^ jnp.uint32(int(_H[0, 0, 0]))) << 3).astype(jnp.int32), 8)
    pt, pf, pk = prep_pieces(0, oz)
    tk = drain(pk, 8)
    tt = drain(pt, 16)
    for c in range(2):
        ties = {t: [tt[8 * c + i]] for i, t in enumerate((4, 5, 7, 8, 10, 11, 12, 13) if c == 0 else (0, 2, 3, 5, 6, 8, 9, 11))}
        for i, t in enumerate((3, 6, 9, 13) if c == 0 else (1, 4, 7, 10)):
            ties.setdefault(t, []).append(tk[4 * c + i])
        mm2(c, [], 0, None, ties, oz)
    wait(c_q[0] + c_w2[2:4])
    start([c_h] + c_q[1])
    side = mlp_pieces(pl.multiple_of(MP + 2 * oz, 16), MM, pb32, B_HID)[0]
    tf = drain(pf, 16)
    mm2(2, side, len(side), None, {3 + i: tf[2 * i:2 * i + 2] for i in range(8)}, oz)
    mm2(3, [], 0)
    wait([c_g] + c_w2[4:])
    start(c_kvf[1])
    for b in range(4):
        conv_pieces(0, oz)[0](b)
    mm2(4, [], 0)
    wait([c_h] + c_q[1] + c_kvf[1])
    start(sum(c_kvf[2:], []) + c_q[2])

    def body(j, oz):
        pl.when(j == 1)(lambda: wait(sum(c_kvf[2:], []) + c_q[2]))
        oz = pl.multiple_of(oz, 8)
        r0 = pl.multiple_of(MP + j * MM, 16)
        r1 = pl.multiple_of(MP + (j + 1) * MM, 16)
        first_half(j, r0, oz, [], (0,) * NT)
        mm2 = mlp_pieces(r0, MM, pb32, B_HID)[2]
        inv = conv_pieces(j, oz)[2]
        fwd = conv_pieces(j + 1, oz)[0]
        pt, pf, pk = prep_pieces(j + 1, oz)
        tt = drain(pt, 16)
        side = pk[:4] + pf + pk[4:] + mlp_pieces(r1, MM, pb32, B_HID)[0]
        mm2(0, side, 4, None, [(4 + i, [tt[i]]) for i in range(10)], oz)
        inv(0)
        mm2(1, side, 20, None, [(2 * i, [tt[10 + i]]) for i in range(6)], oz)
        inv(1)
        inv(2)
        mm2(2, side, len(side))
        inv(3)
        mm2(3, [], 0)
        for b in range(4):
            fwd(b)
        mm2(4, [], 0)
        return oz

    oz = pl.multiple_of(jax.lax.fori_loop(0, NCT - 1, body, oz), 8)

    inv = conv_pieces(NCT - 1, oz)[2]
    mm2 = mlp_pieces(S - ME, ME, pb32, B_HID)[2]
    na = (S - ME) // 16
    cuts = list(range(0, na, 8)) + [na]
    c_out = [copy(o_ref.at[j, 0:S - ME], o_hbm.at[0:S - ME, j * CT:(j + 1) * CT]) for j in range(NCT)]
    c_last = [copy(o_ref.at[j, S - ME:S], o_hbm.at[S - ME:S, j * CT:(j + 1) * CT]) for j in range(NCT)]

    def head(j):
        return [combine(j, a0, a1 - a0, p, oz) for a0, a1 in zip(cuts[:-1], cuts[1:]) for p in range(4)]

    side = head(0) + head(1)
    first_half(NCT - 1, S - ME, oz, side, [share(len(side), t, NT - 2) for t in range(NT - 2)] + [0, 0],
               lambda: start(c_out[0:2]))
    side = head(2)
    for b in range(4):
        inv(b, side, share(len(head(2)), b, 4))
    for c in range(NCT):
        side = head(c + 3) if c < 2 else []
        hooks = {1: lambda: start(c_out[2:4]), 3: lambda: start(c_out[4:] + c_last[0:3])}
        mm2(c, side, len(side), hooks.get(c))
        for p in range(4):
            combine(c, na, ME // 16, p, 0)()
    start(c_last[3:])
    wait(c_out + c_last)


@jax.jit
def pallas_parallel_sum__ssm_conv_h3__dense_activation_gelu__prompt_kernel(
        A_q, A_k, A_v, A_shift_k, A_ssm_k, A_ssm_D, B_x, B_w1, B_b1, B_w2, B_b2):
    hb = pl.BlockSpec(memory_space=pltpu.HBM)
    u32, f32, bf = jnp.uint32, jnp.float32, jnp.bfloat16
    mh = max(MP, MM, ME)
    out = pl.pallas_call(
        _kernel,
        out_shape=jax.ShapeDtypeStruct((S, D), A_q.dtype),
        in_specs=[hb] * 12,
        out_specs=hb,
        scratch_shapes=[
            pltpu.VMEM((2 * C_ROWS + 16, CT), bf),
            pltpu.VMEM((NCT, CT, S), bf),
            pltpu.VMEM((NCT, FP, CT), bf),
            pltpu.VMEM((NCT, FP, CT), bf),
            pltpu.VMEM((N2, N1, N1), u32),
            pltpu.VMEM((N2, N1 // 2, 2 * N1), u32),
            pltpu.VMEM((NCT, S, CT), bf),
            pltpu.VMEM((NCT, S // 2, CT), u32),
            pltpu.VMEM((B_ROWS + 8, CT), u32),
            pltpu.VMEM((2, N2, N1 // 2, CT), u32),
            pltpu.VMEM((N2, N1 + 8, CT), u32),
            pltpu.VMEM((N2, 2 * N1 + 8, CT), f32),
            pltpu.VMEM((S, CT), f32),
            pltpu.VMEM((KS, D), bf),
            pltpu.VMEM((D,), bf),
            pltpu.VMEM((F,), bf),
            pltpu.VMEM((D,), bf),
            pltpu.VMEM((NCT, 8, CT), f32),
            pltpu.VMEM((NCT, N2, N1 + 8, CT), f32),
            pltpu.SemaphoreType.DMA((80,)),
        ],
        compiler_params=pltpu.CompilerParams(vmem_limit_bytes=100 * 1024 * 1024),
    )(A_q.reshape(S, D), A_k.reshape(S, D), A_v.reshape(S, D), A_shift_k.T, A_ssm_k, A_ssm_D,
      B_w1.T, B_b1, B_w2, B_b2, jnp.asarray(_G), jnp.asarray(_H))
    return out.reshape(1, S, D)
```

```python
import functools
import numpy as np
import jax
import jax.numpy as jnp
import jax.experimental.pallas as pl
import jax.experimental.pallas.tpu as pltpu

S, D, F, KS = 2048, 640, 1728, 4
FP = 1792
N1, N2 = 128, 16
CT = 128
NCT = D // CT
MP, MM = 448, 320
ME = MM
MID_PLAN = (7, 6, 6, 5, 5, 5, 5, 5, 5, 5, 5, 5, 4, 0)
FC = 256
MH = max(MP, MM, ME) // 2
NT = FP // CT
B_HID = 0
B_A = NT * MH
B_ROWS = B_A + 2 * N2 * 2 * N1
TS = S // 2
C_K, C_V, C_BASE, C_Q = (i * NCT * TS for i in range(4))
C_TIE = 4 * NCT * TS
C_ROWS = C_TIE + 8
assert MP + (NCT - 1) * MM + ME == S


def _dft_consts():
    n1 = np.arange(N1)
    k1 = np.arange(N1)
    g = np.zeros((N2, 2 * N1, N1), np.float64)
    for n2 in range(N2):
        t = N2 * n1 + n2
        ph = np.pi * t[None, :] / (2 * S) - 2 * np.pi * ((t[None, :] * k1[:, None]) % S) / S
        g[n2, :N1] = np.cos(ph)
        g[n2, N1:] = np.sin(ph)
    g = g.reshape(N2, 2, N1 // 8, 8, N1).transpose(0, 2, 1, 3, 4).reshape(N2, 2 * N1, N1)
    h = np.transpose(g, (0, 2, 1)) / S
    h = h.reshape(N2, N1, 2 * N1 // 16, 2, 8).transpose(0, 1, 2, 4, 3).reshape(N2, N1, 2 * N1)
    g = g.reshape(N2, 2 * N1, N1 // 16, 2, 8).transpose(0, 1, 2, 4, 3).reshape(N2, 2 * N1, N1)

    def pack(m):
        u = np.ascontiguousarray(m).astype(jnp.bfloat16).view(np.uint16).astype(np.uint32)
        return u[:, 0::2, :] | (u[:, 1::2, :] << 16)

    return pack(g), pack(h)


_G, _H = _dft_consts()


def _cmul_const(re, im, e):
    e = e % 16
    if e == 0:
        return re, im
    c = float(np.cos(2 * np.pi * e / 16))
    s = float(-np.sin(2 * np.pi * e / 16))
    if e % 2 == 0:
        if c * s > 0:
            return (re - im) * c, (re + im) * c
        return (re + im) * c, (im - re) * c
    return re * c - im * s, re * s + im * c


def _r4(x, sign, rot2=False):
    (ar, ai), (br, bi), (cr, ci), (dr, di) = x
    if not rot2:
        t0r, t0i = ar + cr, ai + ci
        t1r, t1i = ar - cr, ai - ci
    elif sign > 0:
        t0r, t0i = ar + ci, ai - cr
        t1r, t1i = ar - ci, ai + cr
    else:
        t0r, t0i = ar - ci, ai + cr
        t1r, t1i = ar + ci, ai - cr
    t2r, t2i = br + dr, bi + di
    t3r, t3i = br - dr, bi - di
    y0 = (t0r + t2r, t0i + t2i)
    y2 = (t0r - t2r, t0i - t2i)
    ym = (t1r + t3i, t1i - t3r)
    yp = (t1r - t3i, t1i + t3r)
    if sign > 0:
        return [y0, ym, y2, yp]
    return [y0, yp, y2, ym]


def _tw(y, b, c, sign):
    return y if b * c == 4 else _cmul_const(*y, sign * b * c)


def _unpack(u):
    lo = pltpu.bitcast(u << 16, jnp.float32)
    hi = pltpu.bitcast(u & jnp.uint32(0xFFFF0000), jnp.float32)
    return lo, hi


def _pack(x):
    return pltpu.pack_elementwise([x[0:8], x[8:16]], packed_dtype=jnp.bfloat16)


def _gelu(h):
    c0 = float(np.sqrt(2 / np.pi))
    c1 = c0 * 0.044715
    u = h * (c0 + c1 * (h * h))
    hh = 0.5 * h
    return hh + hh * jnp.tanh(u)


def _kernel(q_hbm, k_hbm, v_hbm, sk_hbm, f_hbm, d_hbm, w1_hbm, b1_hbm, w2_hbm, b2_hbm, g_hbm, h_hbm,
            o_hbm,
            pc_ref, f_ref, w1_ref, w2_ref, g32, h32, o_ref, xn32, pb32, r32, b32, w_ref, t_ref,
            sk_ref, d_ref, b1_ref, b2_ref, prm_ref, y_ref, sems):
    bf = jnp.bfloat16
    u32 = jnp.uint32
    pc32, o32, w132, w232 = (r.bitcast(u32) for r in (pc_ref, o_ref, w1_ref, w2_ref))
    asf = lambda x: pltpu.bitcast(x, jnp.float32)
    asbf = lambda x: pltpu.bitcast(x, bf)
    as32 = lambda x: pltpu.bitcast(x, u32)

    nsem = [0]

    def copy(src, dst):
        c = pltpu.make_async_copy(src, dst, sems.at[nsem[0]])
        nsem[0] += 1
        return c

    def q_copies(r0, r1):
        return [copy(q_hbm.at[r0:r1, c * CT:(c + 1) * CT], pc_ref.at[2 * (C_Q + c * TS) + r0:2 * (C_Q + c * TS) + r1])
                for c in range(NCT)]

    c_q0 = q_copies(0, MP)
    c_small = [copy(sk_hbm, sk_ref), copy(d_hbm, d_ref), copy(b1_hbm, b1_ref), copy(b2_hbm, b2_ref)]
    c_w1 = [[copy(w1_hbm.at[f0:f1, c * CT:(c + 1) * CT], w1_ref.at[c, f0:f1]) for c in range(NCT)]
            for f0, f1 in ((0, FC), (FC, 3 * FC), (3 * FC, F))]
    c_w2 = [copy(w2_hbm.at[:, c * CT:(c + 1) * CT], w2_ref.at[c, 0:F]) for c in range(NCT)]
    c_g = copy(g_hbm, g32)
    c_h0 = copy(h_hbm.at[0], h32.at[0])
    c_h = copy(h_hbm.at[1:N2], h32.at[1:N2])
    c_kvf = [[copy(f_hbm.at[j * CT:(j + 1) * CT], f_ref.at[j]),
              copy(k_hbm.at[:, j * CT:(j + 1) * CT], pc_ref.at[2 * (C_K + j * TS):2 * (C_K + (j + 1) * TS)]),
              copy(v_hbm.at[:, j * CT:(j + 1) * CT], pc_ref.at[2 * (C_V + j * TS):2 * (C_V + (j + 1) * TS)])]
             for j in range(NCT)]
    c_q = [q_copies(r0, r1) for r0, r1 in ((MP, MP + MM), (MP + MM, MP + 2 * MM), (MP + 2 * MM, S))]

    def start(cs):
        for c in cs:
            c.start()

    def wait(cs):
        for c in cs:
            c.wait()

    for c in c_q0 + c_w1[0] + c_small + c_w1[1]:
        c.start()

    w1_ref[:, F:FP, :] = jnp.zeros((NCT, FP - F, CT), bf)
    w2_ref[:, F:FP, :] = jnp.zeros((NCT, FP - F, CT), bf)
    for c in c_small:
        c.wait()
    b1 = b1_ref[...].astype(jnp.float32).reshape(1, F)
    b1 = jnp.concatenate([b1, jnp.zeros((1, FP - F), jnp.float32)], axis=1)
    b2 = b2_ref[...].astype(jnp.float32).reshape(1, D)
    dd = d_ref[...].astype(jnp.float32).reshape(1, D)
    skt = sk_ref[...].astype(jnp.float32)
    for j in range(NCT):
        prm_ref[j, 0:KS, :] = skt[:, j * CT:(j + 1) * CT]
        prm_ref[j, KS:KS + 1, :] = dd[:, j * CT:(j + 1) * CT]

    def drain(q, n):
        toks = []
        for _ in range(n):
            if q:
                toks.append(q.pop(0)())
        return toks

    def tie(x, toks, oz):
        if not toks:
            return x
        t = functools.reduce(jnp.bitwise_or, [as32(z) for z in toks]) & oz.astype(u32)
        return x | t

    def share(n, i, parts):
        return -(-(i + 1) * n // parts) + (-i * n // parts)

    def mlp_pieces(r0, m, hid32, hid0):
        h0 = r0 // 2 if isinstance(r0, int) else pl.multiple_of(r0 // 2, 8)
        ng = m // 16

        def resid(c, g):
            x = asbf(pc32[pl.ds(C_Q + c * TS + h0 + 8 * g, 8), :]).astype(jnp.float32)
            return asbf(_pack(x)).astype(jnp.float32)

        def ln_rows(h, n):
            def run():
                u = jnp.concatenate([pc32[pl.ds(C_Q + c * TS + h, n), :] for c in range(NCT)], axis=1)
                x = jnp.concatenate(_unpack(u), axis=0)
                mu = jnp.mean(x, axis=-1, keepdims=True)
                xc = x - mu
                var = jnp.mean(xc * xc, axis=-1, keepdims=True)
                xn = xc * jax.lax.rsqrt(var + 1e-5)
                xn = pltpu.pack_elementwise([xn[0:n], xn[n:2 * n]], packed_dtype=bf)
                for c in range(NCT):
                    xn32[c, pl.ds(h, n), :] = xn[:, c * CT:(c + 1) * CT]
                return xn[n - 8:n, D - CT:]
            return run

        ln = [ln_rows(h0 + 8 * g, 8 * min(2, ng - g)) for g in range(0, ng, 2)]

        def mm1(t, side, n, side_c=(), n_c=0, hook=None):
            xn = [xn32[c, pl.ds(h0, m // 2), :] for c in range(NCT)]
            xn = asbf(jnp.concatenate(xn, axis=1))
            w = asbf(jnp.concatenate([w132[c, t * CT // 2:(t + 1) * CT // 2, :] for c in range(NCT)], axis=1))
            if hook is not None:
                hook()
            hh = jax.lax.dot_general(xn, w, (((1,), (1,)), ((), ())),
                                     preferred_element_type=jnp.float32) + b1[:, t * CT:(t + 1) * CT]
            hh = _gelu(hh)
            hh = [_pack(hh[16 * g:16 * g + 16]) for g in range(ng)]
            out = []
            for g in range(ng):
                hid32[pl.ds(hid0 + t * MH + 8 * g, 8), :] = hh[g]
                drain(side, share(n, g, ng))
                if share(n_c, g, ng):
                    pc32[C_TIE:C_TIE + 8, :] = hh[g]
                    drain(side_c, share(n_c, g, ng))

        def mm2(c, side, n, hook=None, toks=(), oz=None):
            cs = slice(c * CT, (c + 1) * CT)
            hid, w = [], []
            for t in range(NT):
                if t == NT - 2 and hook is not None:
                    hook()
                x = [hid32[pl.ds(hid0 + t * MH + 8 * g, 8), :] for g in range(ng)]
                x[0] = tie(x[0], dict(toks).get(t), oz)
                hid.append(jnp.concatenate([asbf(z) for z in x], axis=0))
                w.append(w232[c, t * CT // 2:(t + 1) * CT // 2, :])
            o = jnp.dot(jnp.concatenate(hid, axis=1), asbf(jnp.concatenate(w, axis=0)),
                        preferred_element_type=jnp.float32)
            o = o + b2[:, cs]
            out = []
            for g in range(ng):
                pc32[pl.ds(C_BASE + c * TS + h0 + 8 * g, 8), :] = _pack(o[16 * g:16 * g + 16] + resid(c, g))
                out += drain(side, share(n, g, ng))
            return out

        return ln, mm1, mm2

    def prep_pieces(j, oz):
        RB = 16
        k32, v32 = (pc32.at[pl.ds(pl.multiple_of(c + j * TS + oz, 8), TS)] for c in (C_K, C_V))

        def prep_k(i):
            def run():
                s = [prm_ref[j, t:t + 1, :] for t in range(KS)]
                memo = {}

                def pk(n2):
                    p = n2 // 2
                    if p not in memo:
                        if p < 0 and i == 0:
                            row = jax.lax.broadcasted_iota(jnp.int32, (RB, CT), 0)
                            memo[p] = [jnp.where(row == 0, 0.0, pltpu.roll(pk(n + N2), 1, 0)) for n in (2 * p, 2 * p + 1)]
                        else:
                            memo[p] = _unpack(k32[pl.ds(8 * RB * i + p, RB, stride=8), :])
                    return memo[p][n2 % 2]

                for p in range(8):
                    vv = _unpack(v32[pl.ds(8 * RB * i + p, RB, stride=8), :])
                    for e in range(2):
                        n2 = 2 * p + e
                        ksh = pk(n2 - 3) * s[3] + pk(n2 - 2) * s[2] + pk(n2 - 1) * s[1] + pk(n2) * s[0]
                        res = _pack(ksh * vv[e])
                        r32[0, n2, pl.ds(RB // 2 * i, RB // 2), :] = res
                        tok = res if n2 == 0 else tok | res
                return tok
            return run

        def prep_t(m):
            def run():
                ft = f_ref[j, :, m * CT:(m + 1) * CT].astype(jnp.float32).T
                for i in range(CT // 8):
                    t_ref[i % 2, 64 * m + 8 * (i // 2):64 * m + 8 * (i // 2) + 8, :] = ft[8 * i:8 * i + 8]
                return ft[CT - 8:]
            return run

        def prep_f(n2):
            def run():
                ft = t_ref[n2 // 8, pl.ds(n2 % 8, N1, stride=8), :]
                if n2 == 0:
                    row = jax.lax.broadcasted_iota(jnp.int32, (N1, CT), 0)
                    ft = ft + jnp.where(row == 0, prm_ref[j, KS:KS + 1, :], 0.0)
                for g in range(N1 // 16):
                    r32[1, n2, 8 * g:8 * g + 8, :] = _pack(ft[16 * g:16 * g + 16])
                return ft[N1 - 8:]
            return run

        return ([prep_t(m) for m in range(S // CT)], [prep_f(n) for n in range(N2)],
                [prep_k(i) for i in range(N1 // RB)])

    def conv_pieces(j, oz):
        def arow(z, n, r):
            return B_A + (z * N2 + n) * 2 * N1 + 16 * r

        def fwd(b):
            for z in range(2):
                x = [jnp.dot(asbf(g32[4 * a + b]), asbf(r32[z, 4 * a + b]), preferred_element_type=jnp.float32)
                     for a in range(4)]
                for r in range(N1 // 8):
                    y = _r4([(x[a][16 * r:16 * r + 8], x[a][16 * r + 8:16 * r + 16]) for a in range(4)], 1)
                    for c in range(4):
                        yr, yi = _tw(y[c], b, c, 1)
                        pb32[pl.ds(arow(z, 4 * c + b, r), 8), :] = as32(yr)
                        pb32[pl.ds(arow(z, 4 * c + b, r) + 8, 8), :] = as32(yi)

        def mid(c, r):
            zx, zk = (_r4([(asf(pb32[pl.ds(oz + arow(z, 4 * c + b, r), 8), :]),
                            asf(pb32[pl.ds(oz + arow(z, 4 * c + b, r) + 8, 8), :])) for b in range(4)], 1,
                          rot2=(c == 2)) for z in range(2))
            yy = [(xr * kr - xi * ki, xr * ki + xi * kr) for (xr, xi), (kr, ki) in zip(zx, zk)]
            u = _r4(yy, -1)
            for b in range(4):
                ur, ui = _tw(u[b], b, c, -1)
                w_ref[4 * b + c, 16 * r:16 * r + 8, :] = ur
                w_ref[4 * b + c, 16 * r + 8:16 * r + 16, :] = ui

        def last(b, r):
            z = _r4([(w_ref[4 * b + c, pl.ds(oz + 16 * r, 8), :], w_ref[4 * b + c, pl.ds(oz + 16 * r + 8, 8), :])
                     for c in range(4)], -1, rot2=(b == 2))
            for a in range(4):
                b32[4 * a + b, 8 * r:8 * r + 8, :] = pltpu.pack_elementwise(list(z[a]), packed_dtype=bf)

        def spectrum(i):
            def run():
                if i >= 4:
                    last(i % 4, i // 4 - 1)
                if i < 64:
                    mid(i % 4, i // 4)
            return run

        def inv(b, side=(), n=0):
            o = [jnp.dot(asbf(h32[4 * a + b]), asbf(b32[4 * a + b, pl.ds(oz, N1), :]),
                         preferred_element_type=jnp.float32) for a in range(4)]
            for g in range(8):
                for a in range(4):
                    y_ref[j, 4 * a + b, 16 * g:16 * g + 16, :] = o[a][16 * g:16 * g + 16]
                drain(side, share(n, g, 8))

        return fwd, [spectrum(i) for i in range(68)], inv

    def combine(j, a, n, u, oz):
        def run():
            e = 8 * (u // 2) + 2 * (u % 2)
            rows = lambda w: pl.ds(8 * a + w, n, stride=8)
            base = pc32.at[pl.ds(oz + C_BASE + j * TS, TS)]
            b0, b1 = (_unpack(base[rows(2 * (e % 8 + i) + e // 8), :]) for i in range(2))
            for z in range(2):
                n2 = e + 4 * z
                x_lo, x_hi = _unpack(xn32[j, rows(n2 // 2), :])
                o_lo = b0[z] + x_lo * y_ref[j, n2, pl.ds(oz + a, n), :]
                o_hi = b1[z] + x_hi * y_ref[j, n2 + 1, pl.ds(oz + a, n), :]
                o32[j, rows(n2 // 2), :] = pltpu.pack_elementwise([o_lo, o_hi], packed_dtype=bf)
        return run

    def first_half(j, r0, oz, side_c, plan_c, hook=None):
        side = conv_pieces(j, oz)[1]
        mm1 = mlp_pieces(r0, MM, pb32, B_HID)[1]
        for t, n in enumerate(MID_PLAN):
            mm1(t, side, n, side_c, plan_c[t], hook if t == NT - 1 else None)

    ln, mm1, mm2 = mlp_pieces(0, MP, pb32, B_HID)
    wait(c_q0)
    start(c_w1[2])
    drain(ln, 1 << 20)
    for i, ts in enumerate((range(0, 2), range(2, 6), range(6, NT))):
        wait(c_w1[i])
        start((c_w2[:2] + c_kvf[0][:1], c_kvf[0][1:] + [c_h0], c_q[0] + c_w2[2:4])[i])
        for t in ts:
            mm1(t, [], 0)
    wait(c_w2[:2] + c_kvf[0] + [c_h0])
    start([c_g] + c_w2[4:])
    oz = pl.multiple_of(((h32[0, 0, 0] ^ jnp.uint32(int(_H[0, 0, 0]))) << 3).astype(jnp.int32), 8)
    pt, pf, pk = prep_pieces(0, oz)
    tk = drain(pk, 8)
    tt = drain(pt, 16)
    for c in range(2):
        ties = {t: [tt[8 * c + i]] for i, t in enumerate((4, 5, 7, 8, 10, 11, 12, 13) if c == 0 else (0, 2, 3, 5, 6, 8, 9, 11))}
        for i, t in enumerate((3, 6, 9, 13) if c == 0 else (1, 4, 7, 10)):
            ties.setdefault(t, []).append(tk[4 * c + i])
        mm2(c, [], 0, None, ties, oz)
    wait(c_q[0] + c_w2[2:4])
    start([c_h] + c_q[1])
    side = mlp_pieces(pl.multiple_of(MP + 2 * oz, 16), MM, pb32, B_HID)[0]
    tf = drain(pf, 16)
    mm2(2, side, len(side), None, {3 + i: tf[2 * i:2 * i + 2] for i in range(8)}, oz)
    mm2(3, [], 0)
    wait([c_g] + c_w2[4:])
    start(c_kvf[1])
    for b in range(4):
        conv_pieces(0, oz)[0](b)
    mm2(4, [], 0)
    wait([c_h] + c_q[1] + c_kvf[1])
    start(sum(c_kvf[2:], []) + c_q[2])

    def body(j, oz):
        pl.when(j == 1)(lambda: wait(sum(c_kvf[2:], []) + c_q[2]))
        oz = pl.multiple_of(oz, 8)
        r0 = pl.multiple_of(MP + j * MM, 16)
        r1 = pl.multiple_of(MP + (j + 1) * MM, 16)
        first_half(j, r0, oz, [], (0,) * NT)
        mm2 = mlp_pieces(r0, MM, pb32, B_HID)[2]
        inv = conv_pieces(j, oz)[2]
        fwd = conv_pieces(j + 1, oz)[0]
        pt, pf, pk = prep_pieces(j + 1, oz)
        tt = drain(pt, 16)
        tk = drain(pk, 8)
        tf = drain(pf, 16)
        ties = {t: [tt[t]] for t in range(NT)}
        ties[NT - 1] += tt[NT:]
        for i, t in enumerate((3, 7, 11)):
            ties[t].append(tk[i])
        mm2(0, [], 0, None, ties, oz)
        inv(0)
        side = mlp_pieces(r1, MM, pb32, B_HID)[0]
        mm2(1, side, len(side), None, {t: [tk[3 + i]] for i, t in enumerate((0, 4, 8, 12))}, oz)
        inv(1)
        inv(2)
        inv(3)
        ties = {3 + i: tf[2 * i:2 * i + 2] for i in range(8)}
        ties[0] = [tk[7]]
        mm2(2, [], 0, None, ties, oz)
        fwd(0)
        fwd(1)
        mm2(3, [], 0)
        fwd(2)
        fwd(3)
        mm2(4, [], 0)
        return oz

    oz = pl.multiple_of(jax.lax.fori_loop(0, NCT - 1, body, oz), 8)

    inv = conv_pieces(NCT - 1, oz)[2]
    mm2 = mlp_pieces(S - ME, ME, pb32, B_HID)[2]
    na = (S - ME) // 16
    cuts = list(range(0, na, 8)) + [na]
    c_out = [copy(o_ref.at[j, 0:S - ME], o_hbm.at[0:S - ME, j * CT:(j + 1) * CT]) for j in range(NCT)]
    c_last = [copy(o_ref.at[j, S - ME:S], o_hbm.at[S - ME:S, j * CT:(j + 1) * CT]) for j in range(NCT)]

    def head(j):
        return [combine(j, a0, a1 - a0, p, oz) for a0, a1 in zip(cuts[:-1], cuts[1:]) for p in range(4)]

    side = head(0) + head(1)
    first_half(NCT - 1, S - ME, oz, side, [share(len(side), t, NT - 2) for t in range(NT - 2)] + [0, 0],
               lambda: start(c_out[0:2]))
    side = head(2)
    for b in range(4):
        inv(b, side, share(len(head(2)), b, 4))
    for c in range(NCT):
        side = head(c + 3) if c < 2 else []
        hooks = {1: lambda: start(c_out[2:4]), 3: lambda: start(c_out[4:] + c_last[0:3])}
        mm2(c, side, len(side), hooks.get(c))
        for p in range(4):
            combine(c, na, ME // 16, p, 0)()
    start(c_last[3:])
    wait(c_out + c_last)


@jax.jit
def pallas_parallel_sum__ssm_conv_h3__dense_activation_gelu__prompt_kernel(
        A_q, A_k, A_v, A_shift_k, A_ssm_k, A_ssm_D, B_x, B_w1, B_b1, B_w2, B_b2):
    hb = pl.BlockSpec(memory_space=pltpu.HBM)
    u32, f32, bf = jnp.uint32, jnp.float32, jnp.bfloat16
    mh = max(MP, MM, ME)
    out = pl.pallas_call(
        _kernel,
        out_shape=jax.ShapeDtypeStruct((S, D), A_q.dtype),
        in_specs=[hb] * 12,
        out_specs=hb,
        scratch_shapes=[
            pltpu.VMEM((2 * C_ROWS + 16, CT), bf),
            pltpu.VMEM((NCT, CT, S), bf),
            pltpu.VMEM((NCT, FP, CT), bf),
            pltpu.VMEM((NCT, FP, CT), bf),
            pltpu.VMEM((N2, N1, N1), u32),
            pltpu.VMEM((N2, N1 // 2, 2 * N1), u32),
            pltpu.VMEM((NCT, S, CT), bf),
            pltpu.VMEM((NCT, S // 2, CT), u32),
            pltpu.VMEM((B_ROWS + 8, CT), u32),
            pltpu.VMEM((2, N2, N1 // 2, CT), u32),
            pltpu.VMEM((N2, N1 + 8, CT), u32),
            pltpu.VMEM((N2, 2 * N1 + 8, CT), f32),
            pltpu.VMEM((2, S // 2, CT), f32),
            pltpu.VMEM((KS, D), bf),
            pltpu.VMEM((D,), bf),
            pltpu.VMEM((F,), bf),
            pltpu.VMEM((D,), bf),
            pltpu.VMEM((NCT, 8, CT), f32),
            pltpu.VMEM((NCT, N2, N1 + 8, CT), f32),
            pltpu.SemaphoreType.DMA((80,)),
        ],
        compiler_params=pltpu.CompilerParams(vmem_limit_bytes=100 * 1024 * 1024),
    )(A_q.reshape(S, D), A_k.reshape(S, D), A_v.reshape(S, D), A_shift_k.T, A_ssm_k, A_ssm_D,
      B_w1.T, B_b1, B_w2, B_b2, jnp.asarray(_G), jnp.asarray(_H))
    return out.reshape(1, S, D)
```

```python
import functools
import numpy as np
import jax
import jax.numpy as jnp
import jax.experimental.pallas as pl
import jax.experimental.pallas.tpu as pltpu

S, D, F, KS = 2048, 640, 1728, 4
FP = 1792
N1, N2 = 128, 16
CT = 128
NCT = D // CT
MP, MM = 448, 320
ME = MM
PLAN_LOOP = (5, 5, 5, 5, 5, 5, 5, 5, 5, 5, 5, 5, 5, 3)
PLAN_LAST = (7, 6, 6, 5, 5, 5, 5, 5, 5, 5, 5, 5, 4, 0)
FC = 256
MH = max(MP, MM, ME) // 2
NT = FP // CT
B_HID = 0
B_A = NT * MH
B_ROWS = B_A + 2 * N2 * 2 * N1
TS = S // 2
C_K, C_V, C_BASE, C_Q = (i * NCT * TS for i in range(4))
C_TIE = 4 * NCT * TS
C_ROWS = C_TIE + 8
assert MP + (NCT - 1) * MM + ME == S


def _dft_consts():
    n1 = np.arange(N1)
    k1 = np.arange(N1)
    g = np.zeros((N2, 2 * N1, N1), np.float64)
    for n2 in range(N2):
        t = N2 * n1 + n2
        ph = np.pi * t[None, :] / (2 * S) - 2 * np.pi * ((t[None, :] * k1[:, None]) % S) / S
        g[n2, :N1] = np.cos(ph)
        g[n2, N1:] = np.sin(ph)
    g = g.reshape(N2, 2, N1 // 8, 8, N1).transpose(0, 2, 1, 3, 4).reshape(N2, 2 * N1, N1)
    h = np.transpose(g, (0, 2, 1)) / S
    h = h.reshape(N2, N1, 2 * N1 // 16, 2, 8).transpose(0, 1, 2, 4, 3).reshape(N2, N1, 2 * N1)
    g = g.reshape(N2, 2 * N1, N1 // 16, 2, 8).transpose(0, 1, 2, 4, 3).reshape(N2, 2 * N1, N1)

    def pack(m):
        u = np.ascontiguousarray(m).astype(jnp.bfloat16).view(np.uint16).astype(np.uint32)
        return u[:, 0::2, :] | (u[:, 1::2, :] << 16)

    return pack(g), pack(h)


_G, _H = _dft_consts()


def _cmul_const(re, im, e):
    e = e % 16
    if e == 0:
        return re, im
    c = float(np.cos(2 * np.pi * e / 16))
    s = float(-np.sin(2 * np.pi * e / 16))
    if e % 2 == 0:
        if c * s > 0:
            return (re - im) * c, (re + im) * c
        return (re + im) * c, (im - re) * c
    return re * c - im * s, re * s + im * c


def _r4(x, sign, rot2=False):
    (ar, ai), (br, bi), (cr, ci), (dr, di) = x
    if not rot2:
        t0r, t0i = ar + cr, ai + ci
        t1r, t1i = ar - cr, ai - ci
    elif sign > 0:
        t0r, t0i = ar + ci, ai - cr
        t1r, t1i = ar - ci, ai + cr
    else:
        t0r, t0i = ar - ci, ai + cr
        t1r, t1i = ar + ci, ai - cr
    t2r, t2i = br + dr, bi + di
    t3r, t3i = br - dr, bi - di
    y0 = (t0r + t2r, t0i + t2i)
    y2 = (t0r - t2r, t0i - t2i)
    ym = (t1r + t3i, t1i - t3r)
    yp = (t1r - t3i, t1i + t3r)
    if sign > 0:
        return [y0, ym, y2, yp]
    return [y0, yp, y2, ym]


def _tw(y, b, c, sign):
    return y if b * c == 4 else _cmul_const(*y, sign * b * c)


def _unpack(u):
    lo = pltpu.bitcast(u << 16, jnp.float32)
    hi = pltpu.bitcast(u & jnp.uint32(0xFFFF0000), jnp.float32)
    return lo, hi


def _pack(x):
    return pltpu.pack_elementwise([x[0:8], x[8:16]], packed_dtype=jnp.bfloat16)


def _gelu2(h):
    c0 = float(np.sqrt(2 / np.pi))
    c1 = c0 * 0.044715
    u = h * (c0 + c1 * (h * h))
    return h + h * jnp.tanh(u)


def _kernel(q_hbm, k_hbm, v_hbm, sk_hbm, f_hbm, d_hbm, w1_hbm, b1_hbm, w2_hbm, b2_hbm, g_hbm, h_hbm,
            o_hbm,
            pc_ref, f_ref, w1_ref, w2_ref, g32, h32, o_ref, xn32, pb32, r32, b32, w_ref, t_ref,
            sk_ref, d_ref, b1_ref, b2_ref, prm_ref, y_ref, sems):
    bf = jnp.bfloat16
    u32 = jnp.uint32
    pc32, o32, w132, w232 = (r.bitcast(u32) for r in (pc_ref, o_ref, w1_ref, w2_ref))
    asf = lambda x: pltpu.bitcast(x, jnp.float32)
    asbf = lambda x: pltpu.bitcast(x, bf)
    as32 = lambda x: pltpu.bitcast(x, u32)

    nsem = [0]

    def copy(src, dst):
        c = pltpu.make_async_copy(src, dst, sems.at[nsem[0]])
        nsem[0] += 1
        return c

    def q_copies(r0, r1):
        return [copy(q_hbm.at[r0:r1, c * CT:(c + 1) * CT], pc_ref.at[2 * (C_Q + c * TS) + r0:2 * (C_Q + c * TS) + r1])
                for c in range(NCT)]

    c_q0 = q_copies(0, MP)
    c_small = [copy(sk_hbm, sk_ref), copy(d_hbm, d_ref), copy(b1_hbm, b1_ref), copy(b2_hbm, b2_ref)]
    c_w1 = [[copy(w1_hbm.at[f0:f1, c * CT:(c + 1) * CT], w1_ref.at[c, f0:f1]) for c in range(NCT)]
            for f0, f1 in ((0, FC), (FC, 3 * FC), (3 * FC, F))]
    c_w2 = [copy(w2_hbm.at[:, c * CT:(c + 1) * CT], w2_ref.at[c, 0:F]) for c in range(NCT)]
    c_g = copy(g_hbm, g32)
    c_h0 = copy(h_hbm.at[0], h32.at[0])
    c_h = copy(h_hbm.at[1:N2], h32.at[1:N2])
    c_kvf = [[copy(f_hbm.at[j * CT:(j + 1) * CT], f_ref.at[j]),
              copy(k_hbm.at[:, j * CT:(j + 1) * CT], pc_ref.at[2 * (C_K + j * TS):2 * (C_K + (j + 1) * TS)]),
              copy(v_hbm.at[:, j * CT:(j + 1) * CT], pc_ref.at[2 * (C_V + j * TS):2 * (C_V + (j + 1) * TS)])]
             for j in range(NCT)]
    c_q = [q_copies(r0, r1) for r0, r1 in ((MP, MP + MM), (MP + MM, MP + 2 * MM), (MP + 2 * MM, S))]

    def start(cs):
        for c in cs:
            c.start()

    def wait(cs):
        for c in cs:
            c.wait()

    for c in c_q0 + c_w1[0] + c_small + c_w1[1]:
        c.start()

    w1_ref[:, F:FP, :] = jnp.zeros((NCT, FP - F, CT), bf)
    w2_ref[:, F:FP, :] = jnp.zeros((NCT, FP - F, CT), bf)
    for c in c_small:
        c.wait()
    b1 = b1_ref[...].astype(jnp.float32).reshape(1, F)
    b1 = jnp.concatenate([b1, jnp.zeros((1, FP - F), jnp.float32)], axis=1)
    b2 = b2_ref[...].astype(jnp.float32).reshape(1, D)
    dd = d_ref[...].astype(jnp.float32).reshape(1, D)
    skt = sk_ref[...].astype(jnp.float32)
    for j in range(NCT):
        prm_ref[j, 0:KS, :] = skt[:, j * CT:(j + 1) * CT]
        prm_ref[j, KS:KS + 1, :] = dd[:, j * CT:(j + 1) * CT]

    def drain(q, n):
        toks = []
        for _ in range(n):
            if q:
                toks.append(q.pop(0)())
        return toks

    def tie(x, toks, oz):
        if not toks:
            return x
        t = functools.reduce(jnp.bitwise_or, [as32(z) for z in toks]) & oz.astype(u32)
        return x | t

    def share(n, i, parts):
        return -(-(i + 1) * n // parts) + (-i * n // parts)

    def mlp_pieces(r0, m, hid32, hid0):
        h0 = r0 // 2 if isinstance(r0, int) else pl.multiple_of(r0 // 2, 8)
        ng = m // 16

        def resid(c, g):
            x = asbf(pc32[pl.ds(C_Q + c * TS + h0 + 8 * g, 8), :]).astype(jnp.float32)
            return asbf(_pack(x)).astype(jnp.float32)

        def ln_rows(h, n):
            def run():
                u = jnp.concatenate([pc32[pl.ds(C_Q + c * TS + h, n), :] for c in range(NCT)], axis=1)
                x = jnp.concatenate(_unpack(u), axis=0)
                mu = jnp.mean(x, axis=-1, keepdims=True)
                xc = x - mu
                var = jnp.mean(xc * xc, axis=-1, keepdims=True)
                xn = xc * jax.lax.rsqrt(var + 1e-5)
                xn = pltpu.pack_elementwise([xn[0:n], xn[n:2 * n]], packed_dtype=bf)
                for c in range(NCT):
                    xn32[c, pl.ds(h, n), :] = xn[:, c * CT:(c + 1) * CT]
                return xn[n - 8:n, D - CT:]
            return run

        ln = [ln_rows(h0 + 8 * g, 8 * min(2, ng - g)) for g in range(0, ng, 2)]

        def mm1(t, side, n, side_c=(), n_c=0, hook=None):
            xn = [xn32[c, pl.ds(h0, m // 2), :] for c in range(NCT)]
            xn = asbf(jnp.concatenate(xn, axis=1))
            w = asbf(jnp.concatenate([w132[c, t * CT // 2:(t + 1) * CT // 2, :] for c in range(NCT)], axis=1))
            if hook is not None:
                hook()
            hh = jax.lax.dot_general(xn, w, (((1,), (1,)), ((), ())),
                                     preferred_element_type=jnp.float32) + b1[:, t * CT:(t + 1) * CT]
            hh = _gelu2(hh)
            hh = [_pack(hh[16 * g:16 * g + 16]) for g in range(ng)]
            out = []
            for g in range(ng):
                hid32[pl.ds(hid0 + t * MH + 8 * g, 8), :] = hh[g]
                drain(side, share(n, g, ng))
                if share(n_c, g, ng):
                    pc32[C_TIE:C_TIE + 8, :] = hh[g]
                    drain(side_c, share(n_c, g, ng))

        def mm2(c, side, n, hook=None, toks=(), oz=None):
            cs = slice(c * CT, (c + 1) * CT)
            hid, w = [], []
            for t in range(NT):
                if t == NT - 2 and hook is not None:
                    hook()
                x = [hid32[pl.ds(hid0 + t * MH + 8 * g, 8), :] for g in range(ng)]
                x[0] = tie(x[0], dict(toks).get(t), oz)
                hid.append(jnp.concatenate([asbf(z) for z in x], axis=0))
                w.append(w232[c, t * CT // 2:(t + 1) * CT // 2, :])
            o = jnp.dot(jnp.concatenate(hid, axis=1), asbf(jnp.concatenate(w, axis=0)),
                        preferred_element_type=jnp.float32)
            o = 0.5 * o + b2[:, cs]
            out = []
            for g in range(ng):
                pc32[pl.ds(C_BASE + c * TS + h0 + 8 * g, 8), :] = _pack(o[16 * g:16 * g + 16] + resid(c, g))
                out += drain(side, share(n, g, ng))
            return out

        return ln, mm1, mm2

    def prep_pieces(j, oz):
        RB = 16
        k32, v32 = (pc32.at[pl.ds(pl.multiple_of(c + j * TS + oz, 8), TS)] for c in (C_K, C_V))

        def prep_k(i):
            def run():
                s = [prm_ref[j, t:t + 1, :] for t in range(KS)]
                memo = {}

                def pk(n2):
                    p = n2 // 2
                    if p not in memo:
                        if p < 0 and i == 0:
                            row = jax.lax.broadcasted_iota(jnp.int32, (RB, CT), 0)
                            memo[p] = [jnp.where(row == 0, 0.0, pltpu.roll(pk(n + N2), 1, 0)) for n in (2 * p, 2 * p + 1)]
                        else:
                            memo[p] = _unpack(k32[pl.ds(8 * RB * i + p, RB, stride=8), :])
                    return memo[p][n2 % 2]

                for p in range(8):
                    vv = _unpack(v32[pl.ds(8 * RB * i + p, RB, stride=8), :])
                    for e in range(2):
                        n2 = 2 * p + e
                        ksh = pk(n2 - 3) * s[3] + pk(n2 - 2) * s[2] + pk(n2 - 1) * s[1] + pk(n2) * s[0]
                        res = _pack(ksh * vv[e])
                        r32[0, n2, pl.ds(RB // 2 * i, RB // 2), :] = res
                        tok = res if n2 == 0 else tok | res
                return tok
            return run

        def prep_t(m):
            def run():
                ft = f_ref[j, :, m * CT:(m + 1) * CT].astype(jnp.float32).T
                for i in range(CT // 8):
                    t_ref[i % 2, 64 * m + 8 * (i // 2):64 * m + 8 * (i // 2) + 8, :] = ft[8 * i:8 * i + 8]
                return ft[CT - 8:]
            return run

        def prep_f(n2):
            def run():
                ft = t_ref[n2 // 8, pl.ds(n2 % 8, N1, stride=8), :]
                if n2 == 0:
                    row = jax.lax.broadcasted_iota(jnp.int32, (N1, CT), 0)
                    ft = ft + jnp.where(row == 0, prm_ref[j, KS:KS + 1, :], 0.0)
                for g in range(N1 // 16):
                    r32[1, n2, 8 * g:8 * g + 8, :] = _pack(ft[16 * g:16 * g + 16])
                return ft[N1 - 8:]
            return run

        return ([prep_t(m) for m in range(S // CT)], [prep_f(n) for n in range(N2)],
                [prep_k(i) for i in range(N1 // RB)])

    def conv_pieces(j, oz):
        def arow(z, n, r):
            return B_A + (z * N2 + n) * 2 * N1 + 16 * r

        def fwd(b):
            for z in range(2):
                x = [jnp.dot(asbf(g32[4 * a + b]), asbf(r32[z, 4 * a + b]), preferred_element_type=jnp.float32)
                     for a in range(4)]
                for r in range(N1 // 8):
                    y = _r4([(x[a][16 * r:16 * r + 8], x[a][16 * r + 8:16 * r + 16]) for a in range(4)], 1)
                    for c in range(4):
                        yr, yi = _tw(y[c], b, c, 1)
                        pb32[pl.ds(arow(z, 4 * c + b, r), 8), :] = as32(yr)
                        pb32[pl.ds(arow(z, 4 * c + b, r) + 8, 8), :] = as32(yi)

        def mid(c, r):
            zx, zk = (_r4([(asf(pb32[pl.ds(oz + arow(z, 4 * c + b, r), 8), :]),
                            asf(pb32[pl.ds(oz + arow(z, 4 * c + b, r) + 8, 8), :])) for b in range(4)], 1,
                          rot2=(c == 2)) for z in range(2))
            yy = [(xr * kr - xi * ki, xr * ki + xi * kr) for (xr, xi), (kr, ki) in zip(zx, zk)]
            u = _r4(yy, -1)
            for b in range(4):
                ur, ui = _tw(u[b], b, c, -1)
                w_ref[4 * b + c, 16 * r:16 * r + 8, :] = ur
                w_ref[4 * b + c, 16 * r + 8:16 * r + 16, :] = ui

        def last(b, r):
            z = _r4([(w_ref[4 * b + c, pl.ds(oz + 16 * r, 8), :], w_ref[4 * b + c, pl.ds(oz + 16 * r + 8, 8), :])
                     for c in range(4)], -1, rot2=(b == 2))
            for a in range(4):
                b32[4 * a + b, 8 * r:8 * r + 8, :] = pltpu.pack_elementwise(list(z[a]), packed_dtype=bf)

        def spectrum(i):
            def run():
                if i >= 4:
                    last(i % 4, i // 4 - 1)
                if i < 64:
                    mid(i % 4, i // 4)
            return run

        def inv(b, side=(), n=0):
            o = [jnp.dot(asbf(h32[4 * a + b]), asbf(b32[4 * a + b, pl.ds(oz, N1), :]),
                         preferred_element_type=jnp.float32) for a in range(4)]
            for g in range(8):
                for a in range(4):
                    y_ref[j, 4 * a + b, 16 * g:16 * g + 16, :] = o[a][16 * g:16 * g + 16]
                drain(side, share(n, g, 8))

        return fwd, [spectrum(i) for i in range(68)], inv

    def combine(j, a, n, u, oz):
        def run():
            e = 8 * (u // 2) + 2 * (u % 2)
            rows = lambda w: pl.ds(8 * a + w, n, stride=8)
            base = pc32.at[pl.ds(oz + C_BASE + j * TS, TS)]
            b0, b1 = (_unpack(base[rows(2 * (e % 8 + i) + e // 8), :]) for i in range(2))
            for z in range(2):
                n2 = e + 4 * z
                x_lo, x_hi = _unpack(xn32[j, rows(n2 // 2), :])
                o_lo = b0[z] + x_lo * y_ref[j, n2, pl.ds(oz + a, n), :]
                o_hi = b1[z] + x_hi * y_ref[j, n2 + 1, pl.ds(oz + a, n), :]
                o32[j, rows(n2 // 2), :] = pltpu.pack_elementwise([o_lo, o_hi], packed_dtype=bf)
        return run

    def first_half(j, r0, oz, plan, side_c, plan_c, hook=None):
        side = conv_pieces(j, oz)[1]
        mm1 = mlp_pieces(r0, MM, pb32, B_HID)[1]
        for t, n in enumerate(plan):
            mm1(t, side, n, side_c, plan_c[t], hook if t == NT - 1 else None)

    ln, mm1, mm2 = mlp_pieces(0, MP, pb32, B_HID)
    wait(c_q0)
    start(c_w1[2])
    drain(ln, 1 << 20)
    for i, ts in enumerate((range(0, 2), range(2, 6), range(6, NT))):
        wait(c_w1[i])
        start((c_w2[:2] + c_kvf[0][:1], c_kvf[0][1:] + [c_h0], c_q[0] + c_w2[2:4])[i])
        for t in ts:
            mm1(t, [], 0)
    wait(c_w2[:2] + c_kvf[0] + [c_h0])
    start([c_g] + c_w2[4:])
    oz = pl.multiple_of(((h32[0, 0, 0] ^ jnp.uint32(int(_H[0, 0, 0]))) << 3).astype(jnp.int32), 8)
    pt, pf, pk = prep_pieces(0, oz)
    tk = drain(pk, 8)
    tt = drain(pt, 16)
    for c in range(2):
        ties = {t: [tt[8 * c + i]] for i, t in enumerate((4, 5, 7, 8, 10, 11, 12, 13) if c == 0 else (0, 2, 3, 5, 6, 8, 9, 11))}
        for i, t in enumerate((3, 6, 9, 13) if c == 0 else (1, 4, 7, 10)):
            ties.setdefault(t, []).append(tk[4 * c + i])
        mm2(c, [], 0, None, ties, oz)
    wait(c_q[0] + c_w2[2:4])
    start([c_h] + c_q[1])
    side = mlp_pieces(pl.multiple_of(MP + 2 * oz, 16), MM, pb32, B_HID)[0]
    tf = drain(pf, 16)
    mm2(2, side, len(side), None, {3 + i: tf[2 * i:2 * i + 2] for i in range(8)}, oz)
    mm2(3, [], 0)
    wait([c_g] + c_w2[4:])
    start(c_kvf[1])
    for b in range(4):
        conv_pieces(0, oz)[0](b)
    mm2(4, [], 0)
    wait([c_h] + c_q[1] + c_kvf[1])
    start(sum(c_kvf[2:], []) + c_q[2])

    def body(j, oz):
        pl.when(j == 1)(lambda: wait(sum(c_kvf[2:], []) + c_q[2]))
        oz = pl.multiple_of(oz, 8)
        r0 = pl.multiple_of(MP + j * MM, 16)
        r1 = pl.multiple_of(MP + (j + 1) * MM, 16)
        first_half(j, r0, oz, PLAN_LOOP, [], (0,) * NT)
        mm2 = mlp_pieces(r0, MM, pb32, B_HID)[2]
        inv = conv_pieces(j, oz)[2]
        fwd = conv_pieces(j + 1, oz)[0]
        pt, pf, pk = prep_pieces(j + 1, oz)
        tt = drain(pt, 16)
        tk = drain(pk, 8)
        tf = drain(pf, 16)
        ties = {t: [tt[t]] for t in range(NT)}
        ties[NT - 1] += tt[NT:]
        for i, t in enumerate((3, 7, 11)):
            ties[t].append(tk[i])
        mm2(0, [], 0, None, ties, oz)
        inv(0)
        side = mlp_pieces(r1, MM, pb32, B_HID)[0]
        mm2(1, side, len(side), None, {t: [tk[3 + i]] for i, t in enumerate((0, 4, 8, 12))}, oz)
        inv(1)
        inv(2)
        inv(3)
        ties = {3 + i: tf[2 * i:2 * i + 2] for i in range(8)}
        ties[0] = [tk[7]]
        mm2(2, [], 0, None, ties, oz)
        fwd(0)
        fwd(1)
        mm2(3, [], 0)
        fwd(2)
        fwd(3)
        mm2(4, [], 0)
        return oz

    oz = pl.multiple_of(jax.lax.fori_loop(0, NCT - 1, body, oz), 8)

    inv = conv_pieces(NCT - 1, oz)[2]
    mm2 = mlp_pieces(S - ME, ME, pb32, B_HID)[2]
    na = (S - ME) // 16
    cuts = list(range(0, na, 8)) + [na]
    c_out = [copy(o_ref.at[j, 0:S - ME], o_hbm.at[0:S - ME, j * CT:(j + 1) * CT]) for j in range(NCT)]
    c_last = [copy(o_ref.at[j, S - ME:S], o_hbm.at[S - ME:S, j * CT:(j + 1) * CT]) for j in range(NCT)]

    def head(j):
        return [combine(j, a0, a1 - a0, p, oz) for a0, a1 in zip(cuts[:-1], cuts[1:]) for p in range(4)]

    side = head(0) + head(1)
    first_half(NCT - 1, S - ME, oz, PLAN_LAST, side, [share(len(side), t, NT - 2) for t in range(NT - 2)] + [0, 0],
               lambda: start(c_out[0:2]))
    side = head(2)
    for b in range(4):
        inv(b, side, share(len(head(2)), b, 4))
    for c in range(NCT):
        side = head(c + 3) if c < 2 else []
        hooks = {1: lambda: start(c_out[2:4]), 3: lambda: start(c_out[4:] + c_last[0:3])}
        mm2(c, side, len(side), hooks.get(c))
        for p in range(4):
            combine(c, na, ME // 16, p, 0)()
    start(c_last[3:])
    wait(c_out + c_last)


@jax.jit
def pallas_parallel_sum__ssm_conv_h3__dense_activation_gelu__prompt_kernel(
        A_q, A_k, A_v, A_shift_k, A_ssm_k, A_ssm_D, B_x, B_w1, B_b1, B_w2, B_b2):
    hb = pl.BlockSpec(memory_space=pltpu.HBM)
    u32, f32, bf = jnp.uint32, jnp.float32, jnp.bfloat16
    mh = max(MP, MM, ME)
    out = pl.pallas_call(
        _kernel,
        out_shape=jax.ShapeDtypeStruct((S, D), A_q.dtype),
        in_specs=[hb] * 12,
        out_specs=hb,
        scratch_shapes=[
            pltpu.VMEM((2 * C_ROWS + 16, CT), bf),
            pltpu.VMEM((NCT, CT, S), bf),
            pltpu.VMEM((NCT, FP, CT), bf),
            pltpu.VMEM((NCT, FP, CT), bf),
            pltpu.VMEM((N2, N1, N1), u32),
            pltpu.VMEM((N2, N1 // 2, 2 * N1), u32),
            pltpu.VMEM((NCT, S, CT), bf),
            pltpu.VMEM((NCT, S // 2, CT), u32),
            pltpu.VMEM((B_ROWS + 8, CT), u32),
            pltpu.VMEM((2, N2, N1 // 2, CT), u32),
            pltpu.VMEM((N2, N1 + 8, CT), u32),
            pltpu.VMEM((N2, 2 * N1 + 8, CT), f32),
            pltpu.VMEM((2, S // 2, CT), f32),
            pltpu.VMEM((KS, D), bf),
            pltpu.VMEM((D,), bf),
            pltpu.VMEM((F,), bf),
            pltpu.VMEM((D,), bf),
            pltpu.VMEM((NCT, 8, CT), f32),
            pltpu.VMEM((NCT, N2, N1 + 8, CT), f32),
            pltpu.SemaphoreType.DMA((80,)),
        ],
        compiler_params=pltpu.CompilerParams(vmem_limit_bytes=100 * 1024 * 1024),
    )(A_q.reshape(S, D), A_k.reshape(S, D), A_v.reshape(S, D), A_shift_k.T, A_ssm_k, A_ssm_D,
      B_w1.T, B_b1, B_w2, B_b2, jnp.asarray(_G), jnp.asarray(_H))
    return out.reshape(1, S, D)
```

```python
import functools
import numpy as np
import jax
import jax.numpy as jnp
import jax.experimental.pallas as pl
import jax.experimental.pallas.tpu as pltpu

S, D, F, KS = 2048, 640, 1728, 4
FP = 1792
N1, N2 = 128, 16
CT = 128
NCT = D // CT
MP, MM = 448, 320
ME = MM
PLAN_LOOP = (5, 5, 5, 5, 5, 5, 5, 5, 5, 5, 5, 5, 5, 3)
PLAN_LAST = (7, 6, 6, 5, 5, 5, 5, 5, 5, 5, 5, 5, 4, 0)
FC = 256
MH = max(MP, MM, ME) // 2 + 8
NT = FP // CT
B_HID = 0
B_A = NT * MH
AP = 2 * N1 + 8
B_ROWS = B_A + 2 * N2 * AP
TS = S // 2
C_K, C_V, C_BASE, C_Q = (i * NCT * TS for i in range(4))
C_TIE = 4 * NCT * TS
C_ROWS = C_TIE + 8
assert MP + (NCT - 1) * MM + ME == S


def _dft_consts():
    n1 = np.arange(N1)
    k1 = np.arange(N1)
    g = np.zeros((N2, 2 * N1, N1), np.float64)
    for n2 in range(N2):
        t = N2 * n1 + n2
        ph = np.pi * t[None, :] / (2 * S) - 2 * np.pi * ((t[None, :] * k1[:, None]) % S) / S
        g[n2, :N1] = np.cos(ph)
        g[n2, N1:] = np.sin(ph)
    g = g.reshape(N2, 2, N1 // 8, 8, N1).transpose(0, 2, 1, 3, 4).reshape(N2, 2 * N1, N1)
    h = np.transpose(g, (0, 2, 1)) / S
    h = h.reshape(N2, N1, 2 * N1 // 16, 2, 8).transpose(0, 1, 2, 4, 3).reshape(N2, N1, 2 * N1)
    g = g.reshape(N2, 2 * N1, N1 // 16, 2, 8).transpose(0, 1, 2, 4, 3).reshape(N2, 2 * N1, N1)

    def pack(m):
        u = np.ascontiguousarray(m).astype(jnp.bfloat16).view(np.uint16).astype(np.uint32)
        return u[:, 0::2, :] | (u[:, 1::2, :] << 16)

    return pack(g), pack(h)


_G, _H = _dft_consts()


def _cmul_const(re, im, e):
    e = e % 16
    if e == 0:
        return re, im
    c = float(np.cos(2 * np.pi * e / 16))
    s = float(-np.sin(2 * np.pi * e / 16))
    if e % 2 == 0:
        if c * s > 0:
            return (re - im) * c, (re + im) * c
        return (re + im) * c, (im - re) * c
    return re * c - im * s, re * s + im * c


def _r4(x, sign, rot2=False):
    (ar, ai), (br, bi), (cr, ci), (dr, di) = x
    if not rot2:
        t0r, t0i = ar + cr, ai + ci
        t1r, t1i = ar - cr, ai - ci
    elif sign > 0:
        t0r, t0i = ar + ci, ai - cr
        t1r, t1i = ar - ci, ai + cr
    else:
        t0r, t0i = ar - ci, ai + cr
        t1r, t1i = ar + ci, ai - cr
    t2r, t2i = br + dr, bi + di
    t3r, t3i = br - dr, bi - di
    y0 = (t0r + t2r, t0i + t2i)
    y2 = (t0r - t2r, t0i - t2i)
    ym = (t1r + t3i, t1i - t3r)
    yp = (t1r - t3i, t1i + t3r)
    if sign > 0:
        return [y0, ym, y2, yp]
    return [y0, yp, y2, ym]


def _tw(y, b, c, sign):
    return y if b * c == 4 else _cmul_const(*y, sign * b * c)


def _unpack(u):
    lo = pltpu.bitcast(u << 16, jnp.float32)
    hi = pltpu.bitcast(u & jnp.uint32(0xFFFF0000), jnp.float32)
    return lo, hi


def _pack(x):
    return pltpu.pack_elementwise([x[0:8], x[8:16]], packed_dtype=jnp.bfloat16)


def _gelu2(h):
    c0 = float(np.sqrt(2 / np.pi))
    c1 = c0 * 0.044715
    u = h * (c0 + c1 * (h * h))
    return h + h * jnp.tanh(u)


def _kernel(q_hbm, k_hbm, v_hbm, sk_hbm, f_hbm, d_hbm, w1_hbm, b1_hbm, w2_hbm, b2_hbm, g_hbm, h_hbm,
            o_hbm,
            pc_ref, f_ref, w1_ref, w2_ref, g32, h32, o_ref, xn32, pb32, r32, b32, w_ref, t_ref,
            sk_ref, d_ref, b1_ref, b2_ref, prm_ref, y_ref, sems):
    bf = jnp.bfloat16
    u32 = jnp.uint32
    pc32, o32, w132, w232 = (r.bitcast(u32) for r in (pc_ref, o_ref, w1_ref, w2_ref))
    asf = lambda x: pltpu.bitcast(x, jnp.float32)
    asbf = lambda x: pltpu.bitcast(x, bf)
    as32 = lambda x: pltpu.bitcast(x, u32)

    nsem = [0]

    def copy(src, dst):
        c = pltpu.make_async_copy(src, dst, sems.at[nsem[0]])
        nsem[0] += 1
        return c

    def q_copies(r0, r1):
        return [copy(q_hbm.at[r0:r1, c * CT:(c + 1) * CT], pc_ref.at[2 * (C_Q + c * TS) + r0:2 * (C_Q + c * TS) + r1])
                for c in range(NCT)]

    c_q0 = q_copies(0, MP)
    c_small = [copy(sk_hbm, sk_ref), copy(d_hbm, d_ref), copy(b1_hbm, b1_ref), copy(b2_hbm, b2_ref)]
    c_w1 = [[copy(w1_hbm.at[f0:f1, c * CT:(c + 1) * CT], w1_ref.at[c, f0:f1]) for c in range(NCT)]
            for f0, f1 in ((0, FC), (FC, 3 * FC), (3 * FC, F))]
    c_w2 = [copy(w2_hbm.at[:, c * CT:(c + 1) * CT], w2_ref.at[c, 0:F]) for c in range(NCT)]
    c_g = copy(g_hbm, g32)
    c_h0 = copy(h_hbm.at[0], h32.at[0])
    c_h = copy(h_hbm.at[1:N2], h32.at[1:N2])
    c_kvf = [[copy(f_hbm.at[j * CT:(j + 1) * CT], f_ref.at[j]),
              copy(k_hbm.at[:, j * CT:(j + 1) * CT], pc_ref.at[2 * (C_K + j * TS):2 * (C_K + (j + 1) * TS)]),
              copy(v_hbm.at[:, j * CT:(j + 1) * CT], pc_ref.at[2 * (C_V + j * TS):2 * (C_V + (j + 1) * TS)])]
             for j in range(NCT)]
    c_q = [q_copies(r0, r1) for r0, r1 in ((MP, MP + MM), (MP + MM, MP + 2 * MM), (MP + 2 * MM, S))]

    def start(cs):
        for c in cs:
            c.start()

    def wait(cs):
        for c in cs:
            c.wait()

    for c in c_q0 + c_w1[0] + c_small + c_w1[1]:
        c.start()

    w1_ref[:, F:FP, :] = jnp.zeros((NCT, FP - F, CT), bf)
    w2_ref[:, F:FP, :] = jnp.zeros((NCT, FP - F, CT), bf)
    for c in c_small:
        c.wait()
    b1 = b1_ref[...].astype(jnp.float32).reshape(1, F)
    b1 = jnp.concatenate([b1, jnp.zeros((1, FP - F), jnp.float32)], axis=1)
    b2 = b2_ref[...].astype(jnp.float32).reshape(1, D)
    dd = d_ref[...].astype(jnp.float32).reshape(1, D)
    skt = sk_ref[...].astype(jnp.float32)
    for j in range(NCT):
        prm_ref[j, 0:KS, :] = skt[:, j * CT:(j + 1) * CT]
        prm_ref[j, KS:KS + 1, :] = dd[:, j * CT:(j + 1) * CT]

    def drain(q, n):
        toks = []
        for _ in range(n):
            if q:
                toks.append(q.pop(0)())
        return toks

    def tie(x, toks, oz):
        if not toks:
            return x
        t = functools.reduce(jnp.bitwise_or, [as32(z) for z in toks]) & oz.astype(u32)
        return x | t

    def share(n, i, parts):
        return -(-(i + 1) * n // parts) + (-i * n // parts)

    def mlp_pieces(r0, m, hid32, hid0):
        h0 = r0 // 2 if isinstance(r0, int) else pl.multiple_of(r0 // 2, 8)
        ng = m // 16

        def resid(c, g):
            x = asbf(pc32[pl.ds(C_Q + c * TS + h0 + 8 * g, 8), :]).astype(jnp.float32)
            return asbf(_pack(x)).astype(jnp.float32)

        def ln_rows(h, n):
            def run():
                u = jnp.concatenate([pc32[pl.ds(C_Q + c * TS + h, n), :] for c in range(NCT)], axis=1)
                x = jnp.concatenate(_unpack(u), axis=0)
                mu = jnp.mean(x, axis=-1, keepdims=True)
                xc = x - mu
                var = jnp.mean(xc * xc, axis=-1, keepdims=True)
                xn = xc * jax.lax.rsqrt(var + 1e-5)
                xn = pltpu.pack_elementwise([xn[0:n], xn[n:2 * n]], packed_dtype=bf)
                for c in range(NCT):
                    xn32[c, pl.ds(h, n), :] = xn[:, c * CT:(c + 1) * CT]
                return xn[n - 8:n, D - CT:]
            return run

        ln = [ln_rows(h0 + 8 * g, 8 * min(2, ng - g)) for g in range(0, ng, 2)]

        def mm1(t, side, n, side_c=(), n_c=0, hook=None):
            xn = [xn32[c, pl.ds(h0, m // 2), :] for c in range(NCT)]
            xn = asbf(jnp.concatenate(xn, axis=1))
            w = asbf(jnp.concatenate([w132[c, t * CT // 2:(t + 1) * CT // 2, :] for c in range(NCT)], axis=1))
            if hook is not None:
                hook()
            hh = jax.lax.dot_general(xn, w, (((1,), (1,)), ((), ())),
                                     preferred_element_type=jnp.float32) + b1[:, t * CT:(t + 1) * CT]
            hh = _gelu2(hh)
            hh = [_pack(hh[16 * g:16 * g + 16]) for g in range(ng)]
            out = []
            for g in range(ng):
                hid32[pl.ds(hid0 + t * MH + 8 * g, 8), :] = hh[g]
                drain(side, share(n, g, ng))
                if share(n_c, g, ng):
                    pc32[C_TIE:C_TIE + 8, :] = hh[g]
                    drain(side_c, share(n_c, g, ng))

        def mm2(c, side, n, hook=None, toks=(), oz=None):
            cs = slice(c * CT, (c + 1) * CT)
            hid, w = [], []
            for t in range(NT):
                if t == NT - 2 and hook is not None:
                    hook()
                x = [hid32[pl.ds(hid0 + t * MH + 8 * g, 8), :] for g in range(ng)]
                x[0] = tie(x[0], dict(toks).get(t), oz)
                hid.append(jnp.concatenate([asbf(z) for z in x], axis=0))
                w.append(w232[c, t * CT // 2:(t + 1) * CT // 2, :])
            o = jnp.dot(jnp.concatenate(hid, axis=1), asbf(jnp.concatenate(w, axis=0)),
                        preferred_element_type=jnp.float32)
            o = 0.5 * o + b2[:, cs]
            out = []
            for g in range(ng):
                pc32[pl.ds(C_BASE + c * TS + h0 + 8 * g, 8), :] = _pack(o[16 * g:16 * g + 16] + resid(c, g))
                out += drain(side, share(n, g, ng))
            return out

        return ln, mm1, mm2

    def prep_pieces(j, oz):
        RB = 16
        k32, v32 = (pc32.at[pl.ds(pl.multiple_of(c + j * TS + oz, 8), TS)] for c in (C_K, C_V))

        def prep_k(i):
            def run():
                s = [prm_ref[j, t:t + 1, :] for t in range(KS)]
                memo = {}

                def pk(n2):
                    p = n2 // 2
                    if p not in memo:
                        if p < 0 and i == 0:
                            row = jax.lax.broadcasted_iota(jnp.int32, (RB, CT), 0)
                            memo[p] = [jnp.where(row == 0, 0.0, pltpu.roll(pk(n + N2), 1, 0)) for n in (2 * p, 2 * p + 1)]
                        else:
                            memo[p] = _unpack(k32[pl.ds(8 * RB * i + p, RB, stride=8), :])
                    return memo[p][n2 % 2]

                for p in range(8):
                    vv = _unpack(v32[pl.ds(8 * RB * i + p, RB, stride=8), :])
                    for e in range(2):
                        n2 = 2 * p + e
                        ksh = pk(n2 - 3) * s[3] + pk(n2 - 2) * s[2] + pk(n2 - 1) * s[1] + pk(n2) * s[0]
                        res = _pack(ksh * vv[e])
                        r32[0, n2, pl.ds(RB // 2 * i, RB // 2), :] = res
                        tok = res if n2 == 0 else tok | res
                return tok
            return run

        def prep_t(m):
            def run():
                ft = f_ref[j, :, m * CT:(m + 1) * CT].astype(jnp.float32).T
                for i in range(CT // 8):
                    t_ref[i % 2, 64 * m + 8 * (i // 2):64 * m + 8 * (i // 2) + 8, :] = ft[8 * i:8 * i + 8]
                return ft[CT - 8:]
            return run

        def prep_f(n2):
            def run():
                ft = t_ref[n2 // 8, pl.ds(n2 % 8, N1, stride=8), :]
                if n2 == 0:
                    row = jax.lax.broadcasted_iota(jnp.int32, (N1, CT), 0)
                    ft = ft + jnp.where(row == 0, prm_ref[j, KS:KS + 1, :], 0.0)
                for g in range(N1 // 16):
                    r32[1, n2, 8 * g:8 * g + 8, :] = _pack(ft[16 * g:16 * g + 16])
                return ft[N1 - 8:]
            return run

        return ([prep_t(m) for m in range(S // CT)], [prep_f(n) for n in range(N2)],
                [prep_k(i) for i in range(N1 // RB)])

    def conv_pieces(j, oz):
        def arow(z, n, r):
            return B_A + (z * N2 + n) * AP + 16 * r

        def fwd(b):
            for z in range(2):
                x = [jnp.dot(asbf(g32[4 * a + b]), asbf(r32[z, 4 * a + b, 0:N1 // 2, :]), preferred_element_type=jnp.float32)
                     for a in range(4)]
                for r in range(N1 // 8):
                    y = _r4([(x[a][16 * r:16 * r + 8], x[a][16 * r + 8:16 * r + 16]) for a in range(4)], 1)
                    for c in range(4):
                        yr, yi = _tw(y[c], b, c, 1)
                        pb32[pl.ds(arow(z, 4 * c + b, r), 8), :] = as32(yr)
                        pb32[pl.ds(arow(z, 4 * c + b, r) + 8, 8), :] = as32(yi)

        def mid(c, r):
            zx, zk = (_r4([(asf(pb32[pl.ds(oz + arow(z, 4 * c + b, r), 8), :]),
                            asf(pb32[pl.ds(oz + arow(z, 4 * c + b, r) + 8, 8), :])) for b in range(4)], 1,
                          rot2=(c == 2)) for z in range(2))
            yy = [(xr * kr - xi * ki, xr * ki + xi * kr) for (xr, xi), (kr, ki) in zip(zx, zk)]
            u = _r4(yy, -1)
            for b in range(4):
                ur, ui = _tw(u[b], b, c, -1)
                w_ref[4 * b + c, 16 * r:16 * r + 8, :] = ur
                w_ref[4 * b + c, 16 * r + 8:16 * r + 16, :] = ui

        def last(b, r):
            z = _r4([(w_ref[4 * b + c, pl.ds(oz + 16 * r, 8), :], w_ref[4 * b + c, pl.ds(oz + 16 * r + 8, 8), :])
                     for c in range(4)], -1, rot2=(b == 2))
            for a in range(4):
                b32[4 * a + b, 8 * r:8 * r + 8, :] = pltpu.pack_elementwise(list(z[a]), packed_dtype=bf)

        def spectrum(i):
            def run():
                if i >= 4:
                    last(i % 4, i // 4 - 1)
                if i < 64:
                    mid(i % 4, i // 4)
            return run

        def inv(b, side=(), n=0):
            o = [jnp.dot(asbf(h32[4 * a + b]), asbf(b32[4 * a + b, pl.ds(oz, N1), :]),
                         preferred_element_type=jnp.float32) for a in range(4)]
            for g in range(8):
                for a in range(4):
                    y_ref[j, 4 * a + b, 16 * g:16 * g + 16, :] = o[a][16 * g:16 * g + 16]
                drain(side, share(n, g, 8))

        return fwd, [spectrum(i) for i in range(68)], inv

    def combine(j, a, n, u, oz):
        def run():
            e = 8 * (u // 2) + 2 * (u % 2)
            rows = lambda w: pl.ds(8 * a + w, n, stride=8)
            base = pc32.at[pl.ds(oz + C_BASE + j * TS, TS)]
            b0, b1 = (_unpack(base[rows(2 * (e % 8 + i) + e // 8), :]) for i in range(2))
            for z in range(2):
                n2 = e + 4 * z
                x_lo, x_hi = _unpack(xn32[j, rows(n2 // 2), :])
                o_lo = b0[z] + x_lo * y_ref[j, n2, pl.ds(oz + a, n), :]
                o_hi = b1[z] + x_hi * y_ref[j, n2 + 1, pl.ds(oz + a, n), :]
                o32[j, rows(n2 // 2), :] = pltpu.pack_elementwise([o_lo, o_hi], packed_dtype=bf)
        return run

    def first_half(j, r0, oz, plan, side_c, plan_c, hook=None):
        side = conv_pieces(j, oz)[1]
        mm1 = mlp_pieces(r0, MM, pb32, B_HID)[1]
        for t, n in enumerate(plan):
            mm1(t, side, n, side_c, plan_c[t], hook if t == NT - 1 else None)

    ln, mm1, mm2 = mlp_pieces(0, MP, pb32, B_HID)
    wait(c_q0)
    start(c_w1[2])
    drain(ln, 1 << 20)
    for i, ts in enumerate((range(0, 2), range(2, 6), range(6, NT))):
        wait(c_w1[i])
        start((c_w2[:2] + c_kvf[0][:1], c_kvf[0][1:] + [c_h0], c_q[0] + c_w2[2:4])[i])
        for t in ts:
            mm1(t, [], 0)
    wait(c_w2[:2] + c_kvf[0] + [c_h0])
    start([c_g] + c_w2[4:])
    oz = pl.multiple_of(((h32[0, 0, 0] ^ jnp.uint32(int(_H[0, 0, 0]))) << 3).astype(jnp.int32), 8)
    pt, pf, pk = prep_pieces(0, oz)
    tk = drain(pk, 8)
    tt = drain(pt, 16)
    for c in range(2):
        ties = {t: [tt[8 * c + i]] for i, t in enumerate((4, 5, 7, 8, 10, 11, 12, 13) if c == 0 else (0, 2, 3, 5, 6, 8, 9, 11))}
        for i, t in enumerate((3, 6, 9, 13) if c == 0 else (1, 4, 7, 10)):
            ties.setdefault(t, []).append(tk[4 * c + i])
        mm2(c, [], 0, None, ties, oz)
    wait(c_q[0] + c_w2[2:4])
    start([c_h] + c_q[1])
    side = mlp_pieces(pl.multiple_of(MP + 2 * oz, 16), MM, pb32, B_HID)[0]
    tf = drain(pf, 16)
    mm2(2, side, len(side), None, {3 + i: tf[2 * i:2 * i + 2] for i in range(8)}, oz)
    mm2(3, [], 0)
    wait([c_g] + c_w2[4:])
    start(c_kvf[1])
    for b in range(4):
        conv_pieces(0, oz)[0](b)
    mm2(4, [], 0)
    wait([c_h] + c_q[1] + c_kvf[1])
    start(sum(c_kvf[2:], []) + c_q[2])

    def body(j, oz):
        pl.when(j == 1)(lambda: wait(sum(c_kvf[2:], []) + c_q[2]))
        oz = pl.multiple_of(oz, 8)
        r0 = pl.multiple_of(MP + j * MM, 16)
        r1 = pl.multiple_of(MP + (j + 1) * MM, 16)
        first_half(j, r0, oz, PLAN_LOOP, [], (0,) * NT)
        mm2 = mlp_pieces(r0, MM, pb32, B_HID)[2]
        inv = conv_pieces(j, oz)[2]
        fwd = conv_pieces(j + 1, oz)[0]
        pt, pf, pk = prep_pieces(j + 1, oz)
        tt = drain(pt, 16)
        tk = drain(pk, 8)
        tf = drain(pf, 16)
        ties = {t: [tt[t]] for t in range(NT)}
        ties[NT - 1] += tt[NT:]
        for i, t in enumerate((3, 7, 11)):
            ties[t].append(tk[i])
        mm2(0, [], 0, None, ties, oz)
        inv(0)
        side = mlp_pieces(r1, MM, pb32, B_HID)[0]
        mm2(1, side, len(side), None, {t: [tk[3 + i]] for i, t in enumerate((0, 4, 8, 12))}, oz)
        inv(1)
        inv(2)
        inv(3)
        ties = {3 + i: tf[2 * i:2 * i + 2] for i in range(8)}
        ties[0] = [tk[7]]
        mm2(2, [], 0, None, ties, oz)
        fwd(0)
        fwd(1)
        mm2(3, [], 0)
        fwd(2)
        fwd(3)
        mm2(4, [], 0)
        return oz

    oz = pl.multiple_of(jax.lax.fori_loop(0, NCT - 1, body, oz), 8)

    inv = conv_pieces(NCT - 1, oz)[2]
    mm2 = mlp_pieces(S - ME, ME, pb32, B_HID)[2]
    na = (S - ME) // 16
    cuts = list(range(0, na, 8)) + [na]
    c_out = [copy(o_ref.at[j, 0:S - ME], o_hbm.at[0:S - ME, j * CT:(j + 1) * CT]) for j in range(NCT)]
    c_last = [copy(o_ref.at[j, S - ME:S], o_hbm.at[S - ME:S, j * CT:(j + 1) * CT]) for j in range(NCT)]

    def head(j):
        return [combine(j, a0, a1 - a0, p, oz) for a0, a1 in zip(cuts[:-1], cuts[1:]) for p in range(4)]

    side = head(0) + head(1)
    first_half(NCT - 1, S - ME, oz, PLAN_LAST, side, [share(len(side), t, NT - 2) for t in range(NT - 2)] + [0, 0],
               lambda: start(c_out[0:2]))
    side = head(2)
    for b in range(4):
        inv(b, side, share(len(head(2)), b, 4))
    for c in range(NCT):
        side = head(c + 3) if c < 2 else []
        hooks = {1: lambda: start(c_out[2:4]), 3: lambda: start(c_out[4:] + c_last[0:3])}
        mm2(c, side, len(side), hooks.get(c))
        for p in range(4):
            combine(c, na, ME // 16, p, 0)()
    start(c_last[3:])
    wait(c_out + c_last)


@jax.jit
def pallas_parallel_sum__ssm_conv_h3__dense_activation_gelu__prompt_kernel(
        A_q, A_k, A_v, A_shift_k, A_ssm_k, A_ssm_D, B_x, B_w1, B_b1, B_w2, B_b2):
    hb = pl.BlockSpec(memory_space=pltpu.HBM)
    u32, f32, bf = jnp.uint32, jnp.float32, jnp.bfloat16
    out = pl.pallas_call(
        _kernel,
        out_shape=jax.ShapeDtypeStruct((S, D), A_q.dtype),
        in_specs=[hb] * 12,
        out_specs=hb,
        scratch_shapes=[
            pltpu.VMEM((2 * C_ROWS + 16, CT), bf),
            pltpu.VMEM((NCT, CT, S), bf),
            pltpu.VMEM((NCT, FP + 16, CT), bf),
            pltpu.VMEM((NCT, FP, CT), bf),
            pltpu.VMEM((N2, N1, N1), u32),
            pltpu.VMEM((N2, N1 // 2, 2 * N1), u32),
            pltpu.VMEM((NCT, S, CT), bf),
            pltpu.VMEM((NCT, S // 2 + 8, CT), u32),
            pltpu.VMEM((B_ROWS + 8, CT), u32),
            pltpu.VMEM((2, N2, N1 // 2 + 8, CT), u32),
            pltpu.VMEM((N2, N1 + 8, CT), u32),
            pltpu.VMEM((N2, 2 * N1 + 8, CT), f32),
            pltpu.VMEM((2, S // 2, CT), f32),
            pltpu.VMEM((KS, D), bf),
            pltpu.VMEM((D,), bf),
            pltpu.VMEM((F,), bf),
            pltpu.VMEM((D,), bf),
            pltpu.VMEM((NCT, 8, CT), f32),
            pltpu.VMEM((NCT, N2, N1 + 8, CT), f32),
            pltpu.SemaphoreType.DMA((80,)),
        ],
        compiler_params=pltpu.CompilerParams(vmem_limit_bytes=100 * 1024 * 1024),
    )(A_q.reshape(S, D), A_k.reshape(S, D), A_v.reshape(S, D), A_shift_k.T, A_ssm_k, A_ssm_D,
      B_w1.T, B_b1, B_w2, B_b2, jnp.asarray(_G), jnp.asarray(_H))
    return out.reshape(1, S, D)
```

```python
import functools
import numpy as np
import jax
import jax.numpy as jnp
import jax.experimental.pallas as pl
import jax.experimental.pallas.tpu as pltpu

S, D, F, KS = 2048, 640, 1728, 4
FP = 1792
N1, N2 = 128, 16
CT = 128
NCT = D // CT
MP, MM = 448, 320
ME = MM
PLAN_LOOP = (5, 5, 5, 5, 5, 5, 5, 5, 5, 5, 5, 5, 5, 3)
PLAN_LAST = (7, 6, 6, 5, 5, 5, 5, 5, 5, 5, 5, 5, 4, 0)
FC = 256
MH = max(MP, MM, ME) // 2 + 8
NT = FP // CT
B_HID = 0
B_A = NT * MH
AP = 2 * N1 + 8
B_ROWS = B_A + 2 * N2 * AP
TS = S // 2
C_BASE, C_Q, C_TIE = (i * NCT * TS for i in range(3))
C_ROWS = C_TIE + 8
assert MP + (NCT - 1) * MM + ME == S


def _dft_consts():
    n1 = np.arange(N1)
    k1 = np.arange(N1)
    g = np.zeros((N2, 2 * N1, N1), np.float64)
    for n2 in range(N2):
        t = N2 * n1 + n2
        ph = np.pi * t[None, :] / (2 * S) - 2 * np.pi * ((t[None, :] * k1[:, None]) % S) / S
        g[n2, :N1] = np.cos(ph)
        g[n2, N1:] = np.sin(ph)
    g = g.reshape(N2, 2, N1 // 8, 8, N1).transpose(0, 2, 1, 3, 4).reshape(N2, 2 * N1, N1)
    h = np.transpose(g, (0, 2, 1)) / S

    def pack(m):
        u = np.ascontiguousarray(m).astype(jnp.bfloat16).view(np.uint16).astype(np.uint32)
        return u[:, 0::2, :] | (u[:, 1::2, :] << 16)

    return pack(g), pack(h)


_G, _H = _dft_consts()


def _cmul_const(re, im, e):
    e = e % 16
    if e == 0:
        return re, im
    c = float(np.cos(2 * np.pi * e / 16))
    s = float(-np.sin(2 * np.pi * e / 16))
    if e % 2 == 0:
        if c * s > 0:
            return (re - im) * c, (re + im) * c
        return (re + im) * c, (im - re) * c
    return re * c - im * s, re * s + im * c


def _r4(x, sign, rot2=False):
    (ar, ai), (br, bi), (cr, ci), (dr, di) = x
    if not rot2:
        t0r, t0i = ar + cr, ai + ci
        t1r, t1i = ar - cr, ai - ci
    elif sign > 0:
        t0r, t0i = ar + ci, ai - cr
        t1r, t1i = ar - ci, ai + cr
    else:
        t0r, t0i = ar - ci, ai + cr
        t1r, t1i = ar + ci, ai - cr
    t2r, t2i = br + dr, bi + di
    t3r, t3i = br - dr, bi - di
    y0 = (t0r + t2r, t0i + t2i)
    y2 = (t0r - t2r, t0i - t2i)
    ym = (t1r + t3i, t1i - t3r)
    yp = (t1r - t3i, t1i + t3r)
    if sign > 0:
        return [y0, ym, y2, yp]
    return [y0, yp, y2, ym]


def _tw(y, b, c, sign):
    return y if b * c == 4 else _cmul_const(*y, sign * b * c)


def _unpack(u):
    lo = pltpu.bitcast(u << 16, jnp.float32)
    hi = pltpu.bitcast(u & jnp.uint32(0xFFFF0000), jnp.float32)
    return lo, hi


def _pack(x):
    return pltpu.bitcast(x.astype(jnp.bfloat16), jnp.uint32)


def _gelu2(h):
    c0 = float(np.sqrt(2 / np.pi))
    c1 = c0 * 0.044715
    u = h * (c0 + c1 * (h * h))
    return h + h * jnp.tanh(u)


def _kernel(q_hbm, k_hbm, v_hbm, sk_hbm, f_hbm, d_hbm, w1_hbm, b1_hbm, w2_hbm, b2_hbm, g_hbm, h_hbm,
            o_hbm,
            pc_ref, k_ref, v_ref, f_ref, w1_ref, w2_ref, g32, h32, o_ref, xn32, pb32, r_ref, b32, w_ref, t_ref,
            sk_ref, d_ref, b1_ref, b2_ref, prm_ref, y_ref, sems):
    bf = jnp.bfloat16
    u32 = jnp.uint32
    pc32, k32, v32, w132, w232 = (r.bitcast(u32) for r in (pc_ref, k_ref, v_ref, w1_ref, w2_ref))
    asf = lambda x: pltpu.bitcast(x, jnp.float32)
    asbf = lambda x: pltpu.bitcast(x, bf)
    as32 = lambda x: pltpu.bitcast(x, u32)

    nsem = [0]

    def copy(src, dst):
        c = pltpu.make_async_copy(src, dst, sems.at[nsem[0]])
        nsem[0] += 1
        return c

    def q_copies(r0, r1):
        return [copy(q_hbm.at[r0:r1, c * CT:(c + 1) * CT], pc_ref.at[2 * (C_Q + c * TS) + r0:2 * (C_Q + c * TS) + r1])
                for c in range(NCT)]

    c_q0 = q_copies(0, MP)
    c_small = [copy(sk_hbm, sk_ref), copy(d_hbm, d_ref), copy(b1_hbm, b1_ref), copy(b2_hbm, b2_ref)]
    c_w1 = [[copy(w1_hbm.at[f0:f1, c * CT:(c + 1) * CT], w1_ref.at[c, f0:f1]) for c in range(NCT)]
            for f0, f1 in ((0, FC), (FC, 3 * FC), (3 * FC, F))]
    c_w2 = [copy(w2_hbm.at[:, c * CT:(c + 1) * CT], w2_ref.at[c, 0:F]) for c in range(NCT)]
    c_g = copy(g_hbm, g32)
    c_h0 = copy(h_hbm.at[0], h32.at[0])
    c_h = copy(h_hbm.at[1:N2], h32.at[1:N2])
    c_kvf = [[copy(f_hbm.at[j * CT:(j + 1) * CT], f_ref.at[j]),
              copy(k_hbm.at[:, j * CT:(j + 1) * CT], k_ref.at[j]),
              copy(v_hbm.at[:, j * CT:(j + 1) * CT], v_ref.at[j])]
             for j in range(NCT)]
    c_q = [q_copies(r0, r1) for r0, r1 in ((MP, MP + MM), (MP + MM, MP + 2 * MM), (MP + 2 * MM, S))]

    def start(cs):
        for c in cs:
            c.start()

    def wait(cs):
        for c in cs:
            c.wait()

    for c in c_q0 + c_w1[0] + c_small + c_w1[1]:
        c.start()

    w1_ref[:, F:FP, :] = jnp.zeros((NCT, FP - F, CT), bf)
    w2_ref[:, F:FP, :] = jnp.zeros((NCT, FP - F, CT), bf)
    for c in c_small:
        c.wait()
    b1 = b1_ref[...].astype(jnp.float32).reshape(1, F)
    b1 = jnp.concatenate([b1, jnp.zeros((1, FP - F), jnp.float32)], axis=1)
    b2 = b2_ref[...].astype(jnp.float32).reshape(1, D)
    dd = d_ref[...].astype(jnp.float32).reshape(1, D)
    skt = sk_ref[...].astype(jnp.float32)
    for j in range(NCT):
        prm_ref[j, 0:KS, :] = skt[:, j * CT:(j + 1) * CT]
        prm_ref[j, KS:KS + 1, :] = dd[:, j * CT:(j + 1) * CT]

    def drain(q, n):
        toks = []
        for _ in range(n):
            if q:
                toks.append(q.pop(0)())
        return toks

    def tie(x, toks, oz):
        if not toks:
            return x
        t = functools.reduce(jnp.bitwise_or, [as32(z) for z in toks]) & oz.astype(u32)
        return x | t

    def share(n, i, parts):
        return -(-(i + 1) * n // parts) + (-i * n // parts)

    def mlp_pieces(r0, m, hid32, hid0):
        h0 = r0 // 2 if isinstance(r0, int) else pl.multiple_of(r0 // 2, 8)
        ng = m // 16

        def resid(c, g):
            return asbf(pc32[pl.ds(C_Q + c * TS + h0 + 8 * g, 8), :]).astype(jnp.float32)

        def ln_rows(h, n):
            def run():
                x = jnp.concatenate([asbf(pc32[pl.ds(C_Q + c * TS + h, n), :]).astype(jnp.float32)
                                     for c in range(NCT)], axis=1)
                mu = jnp.mean(x, axis=-1, keepdims=True)
                xc = x - mu
                var = jnp.mean(xc * xc, axis=-1, keepdims=True)
                xn = xc * jax.lax.rsqrt(var + 1e-5)
                for c in range(NCT):
                    xn32[c, pl.ds(h, n), :] = _pack(xn[:, c * CT:(c + 1) * CT])
                return xn[n - 8:n, D - CT:]
            return run

        ln = [ln_rows(h0 + 8 * g, 8 * min(2, ng - g)) for g in range(0, ng, 2)]

        def mm1(t, side, n, side_c=(), n_c=0, hook=None):
            xn = [xn32[c, pl.ds(h0, m // 2), :] for c in range(NCT)]
            xn = asbf(jnp.concatenate(xn, axis=1))
            w = asbf(jnp.concatenate([w132[c, t * CT // 2:(t + 1) * CT // 2, :] for c in range(NCT)], axis=1))
            if hook is not None:
                hook()
            hh = jax.lax.dot_general(xn, w, (((1,), (1,)), ((), ())),
                                     preferred_element_type=jnp.float32) + b1[:, t * CT:(t + 1) * CT]
            hh = _gelu2(hh)
            hh = [_pack(hh[16 * g:16 * g + 16]) for g in range(ng)]
            out = []
            for g in range(ng):
                hid32[pl.ds(hid0 + t * MH + 8 * g, 8), :] = hh[g]
                drain(side, share(n, g, ng))
                if share(n_c, g, ng):
                    pc32[C_TIE:C_TIE + 8, :] = hh[g]
                    drain(side_c, share(n_c, g, ng))

        def mm2(c, side, n, hook=None, toks=(), oz=None):
            cs = slice(c * CT, (c + 1) * CT)
            hid, w = [], []
            for t in range(NT):
                if t == NT - 2 and hook is not None:
                    hook()
                x = [hid32[pl.ds(hid0 + t * MH + 8 * g, 8), :] for g in range(ng)]
                x[0] = tie(x[0], dict(toks).get(t), oz)
                hid.append(jnp.concatenate([asbf(z) for z in x], axis=0))
                w.append(w232[c, t * CT // 2:(t + 1) * CT // 2, :])
            o = jnp.dot(jnp.concatenate(hid, axis=1), asbf(jnp.concatenate(w, axis=0)),
                        preferred_element_type=jnp.float32)
            o = 0.5 * o + b2[:, cs]
            out = []
            for g in range(ng):
                pc32[pl.ds(C_BASE + c * TS + h0 + 8 * g, 8), :] = _pack(o[16 * g:16 * g + 16] + resid(c, g))
                out += drain(side, share(n, g, ng))
            return out

        return ln, mm1, mm2

    def prep_pieces(j, oz):
        RB = 16

        def prep_k(i):
            def run():
                s = [prm_ref[j, t:t + 1, :] for t in range(KS)]
                memo = {}

                def pk(n2):
                    p = n2 // 2
                    if p not in memo:
                        if p < 0 and i == 0:
                            row = jax.lax.broadcasted_iota(jnp.int32, (RB, CT), 0)
                            memo[p] = [jnp.where(row == 0, 0.0, pltpu.roll(pk(n + N2), 1, 0)) for n in (2 * p, 2 * p + 1)]
                        else:
                            memo[p] = _unpack(k32[j, pl.ds(8 * RB * i + p, RB, stride=8), :])
                    return memo[p][n2 % 2]

                for p in range(8):
                    vv = _unpack(v32[j, pl.ds(8 * RB * i + p, RB, stride=8), :])
                    for e in range(2):
                        n2 = 2 * p + e
                        ksh = pk(n2 - 3) * s[3] + pk(n2 - 2) * s[2] + pk(n2 - 1) * s[1] + pk(n2) * s[0]
                        res = ksh * vv[e]
                        r_ref[n2, pl.ds(RB * i, RB), :] = res
                        if e:
                            tok = as32(res[8:]) if p == 0 else tok | as32(res[8:])
                return tok
            return run

        def prep_t(m):
            def run():
                ft = f_ref[j, :, m * CT:(m + 1) * CT].astype(jnp.float32).T
                for i in range(CT // 8):
                    t_ref[i % 2, 64 * m + 8 * (i // 2):64 * m + 8 * (i // 2) + 8, :] = ft[8 * i:8 * i + 8]
                return ft[CT - 8:]
            return run

        return [prep_t(m) for m in range(S // CT)], [prep_k(i) for i in range(N1 // RB)]

    def conv_pieces(j, oz):
        def arow(z, n, r):
            return B_A + (z * N2 + n) * AP + 16 * r

        def operand(z, n2):
            if z == 0:
                return r_ref[n2, 0:N1, :]
            ft = t_ref[n2 // 8, pl.ds(n2 % 8, N1, stride=8), :]
            if n2 == 0:
                row = jax.lax.broadcasted_iota(jnp.int32, (N1, CT), 0)
                ft = ft + jnp.where(row == 0, prm_ref[j, KS:KS + 1, :], 0.0)
            return ft

        def fwd(b):
            for z in range(2):
                x = [jnp.dot(asbf(g32[4 * a + b]), operand(z, 4 * a + b).astype(bf), preferred_element_type=jnp.float32)
                     for a in range(4)]
                for r in range(N1 // 8):
                    y = _r4([(x[a][16 * r:16 * r + 8], x[a][16 * r + 8:16 * r + 16]) for a in range(4)], 1)
                    for c in range(4):
                        yr, yi = _tw(y[c], b, c, 1)
                        pb32[pl.ds(arow(z, 4 * c + b, r), 8), :] = as32(yr)
                        pb32[pl.ds(arow(z, 4 * c + b, r) + 8, 8), :] = as32(yi)

        def mid(c, r):
            zx, zk = (_r4([(asf(pb32[pl.ds(oz + arow(z, 4 * c + b, r), 8), :]),
                            asf(pb32[pl.ds(oz + arow(z, 4 * c + b, r) + 8, 8), :])) for b in range(4)], 1,
                          rot2=(c == 2)) for z in range(2))
            yy = [(xr * kr - xi * ki, xr * ki + xi * kr) for (xr, xi), (kr, ki) in zip(zx, zk)]
            u = _r4(yy, -1)
            for b in range(4):
                ur, ui = _tw(u[b], b, c, -1)
                w_ref[4 * b + c, 16 * r:16 * r + 8, :] = ur
                w_ref[4 * b + c, 16 * r + 8:16 * r + 16, :] = ui

        def last(b, r):
            z = _r4([(w_ref[4 * b + c, pl.ds(oz + 16 * r, 8), :], w_ref[4 * b + c, pl.ds(oz + 16 * r + 8, 8), :])
                     for c in range(4)], -1, rot2=(b == 2))
            for a in range(4):
                b32[4 * a + b, 8 * r:8 * r + 8, :] = _pack(jnp.concatenate(z[a], axis=0))

        def spectrum(i):
            def run():
                if i >= 4:
                    last(i % 4, i // 4 - 1)
                if i < 64:
                    mid(i % 4, i // 4)
            return run

        def inv(b, side=(), n=0):
            o = [jnp.dot(asbf(h32[4 * a + b]), asbf(b32[4 * a + b, pl.ds(oz, N1), :]),
                         preferred_element_type=jnp.float32) for a in range(4)]
            for g in range(8):
                for a in range(4):
                    n2 = 4 * a + b
                    y_ref[j, n2 // 8, pl.ds(128 * g + n2 % 8, 16, stride=8), :] = o[a][16 * g:16 * g + 16]
                drain(side, share(n, g, 8))

        return fwd, [spectrum(i) for i in range(68)], inv

    def combine(c0, c1, g0, g1, oz):
        def run():
            for g in range(g0, g1):
                o = []
                for c in range(c0, c1):
                    base = asbf(pc32[pl.ds(oz + C_BASE + c * TS + 8 * g, 8), :]).astype(jnp.float32)
                    xn = asbf(xn32[c, 8 * g:8 * g + 8, :]).astype(jnp.float32)
                    y = jnp.concatenate([y_ref[c, h, pl.ds(oz + 8 * g, 8), :] for h in range(2)], axis=0)
                    o.append(base + xn * y)
                o_ref[16 * g:16 * g + 16, c0 * CT:c1 * CT] = jnp.concatenate(o, axis=1).astype(bf)
        return run

    def first_half(j, r0, oz, plan, side_c, plan_c, hook=None):
        side = conv_pieces(j, oz)[1]
        mm1 = mlp_pieces(r0, MM, pb32, B_HID)[1]
        for t, n in enumerate(plan):
            mm1(t, side, n, side_c, plan_c[t], hook if t == NT - 1 else None)

    ln, mm1, mm2 = mlp_pieces(0, MP, pb32, B_HID)
    wait(c_q0)
    start(c_w1[2])
    drain(ln, 1 << 20)
    for i, ts in enumerate((range(0, 2), range(2, 6), range(6, NT))):
        wait(c_w1[i])
        start((c_w2[:2] + c_kvf[0][:1], c_kvf[0][1:] + [c_h0], c_q[0] + c_w2[2:4])[i])
        for t in ts:
            mm1(t, [], 0)
    wait(c_w2[:2] + c_kvf[0] + [c_h0])
    start([c_g] + c_w2[4:])
    oz = pl.multiple_of(((h32[0, 0, 0] ^ jnp.uint32(int(_H[0, 0, 0]))) << 3).astype(jnp.int32), 8)
    pt, pk = prep_pieces(0, oz)
    tk = drain(pk, 8)
    tt = drain(pt, 16)
    for c in range(2):
        ties = {t: [tt[8 * c + i]] for i, t in enumerate((4, 5, 7, 8, 10, 11, 12, 13) if c == 0 else (0, 2, 3, 5, 6, 8, 9, 11))}
        for i, t in enumerate((3, 6, 9, 13) if c == 0 else (1, 4, 7, 10)):
            ties.setdefault(t, []).append(tk[4 * c + i])
        mm2(c, [], 0, None, ties, oz)
    wait(c_q[0] + c_w2[2:4])
    start([c_h] + c_q[1])
    side = mlp_pieces(pl.multiple_of(MP + 2 * oz, 16), MM, pb32, B_HID)[0]
    mm2(2, side, len(side))
    mm2(3, [], 0)
    wait([c_g] + c_w2[4:])
    start(c_kvf[1])
    for b in range(4):
        conv_pieces(0, oz)[0](b)
    mm2(4, [], 0)
    wait([c_h] + c_q[1] + c_kvf[1])
    start(sum(c_kvf[2:], []) + c_q[2])

    def body(j, oz):
        pl.when(j == 1)(lambda: wait(sum(c_kvf[2:], []) + c_q[2]))
        oz = pl.multiple_of(oz, 8)
        r0 = pl.multiple_of(MP + j * MM, 16)
        r1 = pl.multiple_of(MP + (j + 1) * MM, 16)
        first_half(j, r0, oz, PLAN_LOOP, [], (0,) * NT)
        mm2 = mlp_pieces(r0, MM, pb32, B_HID)[2]
        inv = conv_pieces(j, oz)[2]
        fwd = conv_pieces(j + 1, oz)[0]
        pt, pk = prep_pieces(j + 1, oz)
        tt = drain(pt, 16)
        tk = drain(pk, 8)
        ties = {t: [tt[t]] for t in range(NT)}
        ties[NT - 1] += tt[NT:]
        for i, t in enumerate((3, 7, 11)):
            ties[t].append(tk[i])
        mm2(0, [], 0, None, ties, oz)
        inv(0)
        side = mlp_pieces(r1, MM, pb32, B_HID)[0]
        mm2(1, side, len(side), None, {t: [tk[3 + i]] for i, t in enumerate((0, 4, 8, 12))}, oz)
        inv(1)
        inv(2)
        inv(3)
        mm2(2, [], 0, None, {2: [tk[7]]}, oz)
        fwd(0)
        fwd(1)
        mm2(3, [], 0)
        fwd(2)
        fwd(3)
        mm2(4, [], 0)
        return oz

    oz = pl.multiple_of(jax.lax.fori_loop(0, NCT - 1, body, oz), 8)

    inv = conv_pieces(NCT - 1, oz)[2]
    mm2 = mlp_pieces(S - ME, ME, pb32, B_HID)[2]
    na = (S - ME) // 16
    groups = ((0, 2), (2, 4), (4, 5))
    c_out, c_last = ([copy(o_ref.at[r0:r1, c0 * CT:c1 * CT], o_hbm.at[r0:r1, c0 * CT:c1 * CT]) for c0, c1 in groups]
                     for r0, r1 in ((0, S - ME), (S - ME, S)))

    def head(i):
        return [combine(*groups[i], g, g + 2, oz) for g in range(0, na, 2)]

    side = head(0)
    first_half(NCT - 1, S - ME, oz, PLAN_LAST, side, [share(len(side), t, NT - 2) for t in range(NT - 2)] + [0, 0],
               c_out[0].start)
    side = head(1)
    for b in range(4):
        inv(b, side, na // 16)
    mm2(0, side, len(side))
    side = head(2)
    mm2(1, side, len(side), c_out[1].start)
    combine(*groups[0], na, S // 16, 0)()
    mm2(2, [], 0)
    mm2(3, [], 0, lambda: start([c_out[2], c_last[0]]))
    combine(*groups[1], na, S // 16, 0)()
    mm2(4, [], 0, c_last[1].start)
    combine(*groups[2], na, S // 16, 0)()
    c_last[2].start()
    wait(c_out + c_last)


@jax.jit
def pallas_parallel_sum__ssm_conv_h3__dense_activation_gelu__prompt_kernel(
        A_q, A_k, A_v, A_shift_k, A_ssm_k, A_ssm_D, B_x, B_w1, B_b1, B_w2, B_b2):
    hb = pl.BlockSpec(memory_space=pltpu.HBM)
    u32, f32, bf = jnp.uint32, jnp.float32, jnp.bfloat16
    out = pl.pallas_call(
        _kernel,
        out_shape=jax.ShapeDtypeStruct((S, D), A_q.dtype),
        in_specs=[hb] * 12,
        out_specs=hb,
        scratch_shapes=[
            pltpu.VMEM((2 * C_ROWS + 16, CT), bf),
            pltpu.VMEM((NCT, S, CT), bf),
            pltpu.VMEM((NCT, S, CT), bf),
            pltpu.VMEM((NCT, CT, S), bf),
            pltpu.VMEM((NCT, FP + 16, CT), bf),
            pltpu.VMEM((NCT, FP, CT), bf),
            pltpu.VMEM((N2, N1, N1), u32),
            pltpu.VMEM((N2, N1 // 2, 2 * N1), u32),
            pltpu.VMEM((S, D), bf),
            pltpu.VMEM((NCT, S // 2 + 8, CT), u32),
            pltpu.VMEM((B_ROWS + 8, CT), u32),
            pltpu.VMEM((N2, N1 + 8, CT), f32),
            pltpu.VMEM((N2, N1 + 8, CT), u32),
            pltpu.VMEM((N2, 2 * N1 + 8, CT), f32),
            pltpu.VMEM((2, S // 2, CT), f32),
            pltpu.VMEM((KS, D), bf),
            pltpu.VMEM((D,), bf),
            pltpu.VMEM((F,), bf),
            pltpu.VMEM((D,), bf),
            pltpu.VMEM((NCT, 8, CT), f32),
            pltpu.VMEM((NCT, 2, S // 2 + 8, CT), f32),
            pltpu.SemaphoreType.DMA((80,)),
        ],
        compiler_params=pltpu.CompilerParams(vmem_limit_bytes=100 * 1024 * 1024),
    )(A_q.reshape(S, D), A_k.reshape(S, D), A_v.reshape(S, D), A_shift_k.T, A_ssm_k, A_ssm_D,
      B_w1.T, B_b1, B_w2, B_b2, jnp.asarray(_G), jnp.asarray(_H))
    return out.reshape(1, S, D)
```
